```python
import jax
import jax.numpy as jnp

def _softmax(x, axis=-1):
    return jax.nn.softmax(x, axis=axis)
def _gelu(x):
    return jax.nn.gelu(x, approximate=True)
def _silu(x):
    return jax.nn.silu(x)
def _sigmoid(x):
    return jax.nn.sigmoid(x)
def _layernorm(x, axis=-1, eps=1e-5):
    m = jnp.mean(x, axis=axis, keepdims=True)
    v = jnp.var(x, axis=axis, keepdims=True)
    return (x - m) / jnp.sqrt(v + eps)
def _scatter_add(tgt, idx, src, axis=0):
    return tgt.at[idx].add(src)
def _segment_sum(src, seg, n):
    return jax.ops.segment_sum(src, seg, n)
class _Rng:
    def __init__(self, key):
        self._k = key
    def _next(self):
        self._k, sub = jax.random.split(self._k)
        return sub
    def normal(self, shape):
        return jax.random.normal(self._next(), shape, dtype=jnp.bfloat16)
    def randint(self, lo, hi, shape):
        return jax.random.randint(self._next(), shape, lo, hi, dtype=jnp.int32)
    def uniform(self, shape, lo=0.0, hi=1.0):
        return jax.random.uniform(self._next(), shape, jnp.bfloat16, lo, hi)
    def permutation(self, n):
        return jax.random.permutation(self._next(), n)


kernel_name = 'gated_mix__sliding_local_dilated__moe_arch_mod__prompt'

def setup_inputs():
    _rng = _Rng(jax.random.key(int.from_bytes(__import__("os").urandom(4), "little")))
    _w = (lambda a: (lambda t: t.astype(jnp.bfloat16) if jnp.issubdtype(t.dtype, jnp.floating) else t)(jnp.asarray(a)))
    def _A_setup():
        B, S, D = 1, 2048, 640
        return {
            "x": _w((lambda *s: _rng.normal(s) * 0.05)(B, S, D)),
            "wqkv": _w((lambda *s: _rng.normal(s) * 0.05)(D, 3 * D)),
            "wo": _w((lambda *s: _rng.normal(s) * 0.05)(D, D)),
        }
    _A_in = _A_setup()

    def _B_setup():
        B, S, D, F, C = 1, 2048, 640, 1728, 2
        return {
            "x": _w((lambda *s: _rng.normal(s) * 0.05)(B, S, D)),
            "w_r": _w((lambda *s: _rng.normal(s) * 0.05)(D)),
            "w_gate": _w((lambda *s: _rng.normal(s) * 0.05)(D, F)),
            "w_up": _w((lambda *s: _rng.normal(s) * 0.05)(D, F)),
            "w_down": _w((lambda *s: _rng.normal(s) * 0.05)(F, D)),
        }
    _B_in = _B_setup()

    return {
        "A_x": _A_in["x"],
        "A_wqkv": _A_in["wqkv"],
        "A_wo": _A_in["wo"],
        "B_x": _B_in["x"],
        "B_w_r": _B_in["w_r"],
        "B_w_gate": _B_in["w_gate"],
        "B_w_up": _B_in["w_up"],
        "B_w_down": _B_in["w_down"],
        "gate_w": _w((lambda *s: _rng.normal(s) * 0.05)(640)),
    }

def reference(A_x, A_wqkv, A_wo, B_x, B_w_r, B_w_gate, B_w_up, B_w_down, gate_w):
    def _A_ref(x, wqkv, wo):
        B, S, D = x.shape
        H = 32; Dh = D // H
        W, dil = 8, 2
        qkv = (lambda x, *d: x.transpose(*d))((x @ wqkv).reshape(B, S, 3, H, Dh), 2, 0, 3, 1, 4)
        q, k, v = qkv[0], qkv[1], qkv[2]
        scale = Dh ** -0.5
        pos = jnp.arange(S)
        off = jnp.arange(W) * dil
        idx = pos[:, None] - off[None, :]
        mask = idx >= 0
        idx_c = jnp.where(mask, idx, 0).reshape(-1)
        kg = k[:, :, idx_c, :].reshape(B, H, S, W, Dh)
        vg = v[:, :, idx_c, :].reshape(B, H, S, W, Dh)
        logits = jnp.einsum("bhsd,bhswd->bhsw", q, kg) * scale
        logits = jnp.where(mask[None, None, :, :], logits, -1e9)
        attn = _softmax(logits, axis=-1)
        o = jnp.einsum("bhsw,bhswd->bhsd", attn, vg)
        return (lambda x, *d: x.transpose(*d))(o, 0, 2, 1, 3).reshape(B, S, D) @ wo

    def _B_ref(x, w_r, w_gate, w_up, w_down):
        B, S, D = x.shape
        C = 2
        r = x @ w_r
        idx = jnp.argsort(-r, axis=-1)[:, :C]
        idx_e = jnp.repeat(idx.reshape(B, C, 1), D, axis=2)
        x_sel = jnp.take_along_axis(x, idx_e, axis=1)
        g = _silu(x_sel @ w_gate)
        u = x_sel @ w_up
        y = (g * u) @ w_down
        r_sel = _sigmoid(jnp.take_along_axis(r, idx, axis=1))
        y = y * r_sel.reshape(B, C, 1)
        b_off = (jnp.arange(B) * S).reshape(B, 1)
        flat_idx = (idx + b_off).reshape(B * C)
        zero = (x * 0.0).reshape(B * S, D)
        upd = _scatter_add(zero, flat_idx, y.reshape(B * C, D), axis=0)
        return x + upd.reshape(B, S, D)

    x = A_x
    g = _sigmoid((x * gate_w).sum(-1, keepdims=True))
    a = _A_ref(x, A_wqkv, A_wo)
    b = _B_ref(x, B_w_r, B_w_gate, B_w_up, B_w_down)
    return g * a + (1 - g) * b
```

```python
import contextlib
import numpy as np
import jax
import jax.numpy as jnp
from jax import lax
from jax.experimental import pallas as pl
from jax.experimental.pallas import tpu as pltpu

S, D, H, DH, W, DIL, F = 2048, 640, 32, 20, 8, 2, 1728
NT = D // 128
HALO = 16
F32, BF16, I32 = jnp.float32, jnp.bfloat16, jnp.int32
HI = np.int32(-65536)


def tree(f, xs):
    while len(xs) > 1:
        xs = [f(xs[k], xs[k + 1]) if k + 1 < len(xs) else xs[k] for k in range(0, len(xs), 2)]
    return xs[0]


def add(a, b):
    return a + b


def make(TM=256, RG=8, TM2=256, flags=None, scopes=False, dl=(6, 6, 6, 4), order=(1, 0, 2),
         xw=(1, 2), ffn_at=6, wo_at=5, lag=0, nwo=3, rt=(1, 2, 3, 4), qktree=True, newton=True):
    NB, NB2 = S // TM, S // TM2
    scope = (lambda n: jax.named_scope("Z" + n)) if scopes else (lambda n: contextlib.nullcontext())

    def kern(ax_hbm, wqkv_hbm, wo_hbm, wr_ref, wg_hbm, wu_hbm, wd_hbm, gw_ref, out_hbm,
             ax, wraw, wp, wo_raw, wo_f32, wop, wg, wu, wd, qkv, o_s, out_s, sx, sw, so):
        ax_h, wqkv_h, out_h = (r.bitcast(I32) for r in (ax_hbm, wqkv_hbm, out_hbm))
        T2 = TM // 2
        xb = [0] + list(xw) + [NB]
        cp_x = [pltpu.make_async_copy(ax_h.at[pl.ds(a * T2, (b - a) * T2)], ax.at[pl.ds(a * T2, (b - a) * T2)], sx.at[k])
                for k, (a, b) in enumerate(zip(xb[:-1], xb[1:]))]
        cp_w = [pltpu.make_async_copy(wqkv_h.at[:, pl.ds(s * D, D)], wraw.at[s], sw.at[s]) for s in range(3)]
        cp_wo = pltpu.make_async_copy(wo_hbm.bitcast(I32), wo_raw, sw.at[3])
        cp_f = [pltpu.make_async_copy(h.bitcast(I32), v, sw.at[4 + k])
                for k, (h, v) in enumerate(((wg_hbm, wg), (wu_hbm, wu), (wd_hbm, wd)))]
        for c in [cp_w[order[0]], cp_x[0], cp_w[order[1]], cp_w[order[2]]] + cp_x[1:] + [cp_wo] + cp_f:
            c.start()

        lane = lax.broadcasted_iota(I32, (8, 128), 1)

        def permute_section(s):
            for jp in range(NT):
                src = (20 * (lane & 31) + 4 * jp + (lane >> 5)) & 127
                tile = (20 * ((13 * ((lane >> 2) - jp)) & 31) + 4 * jp + (lane & 3)) >> 7
                for r in range(D // 16):
                    rows = pl.ds(r * 8, 8)
                    acc = wraw[s, rows, pl.ds(0, 128)]
                    for j in range(1, NT):
                        acc = jnp.where(tile == j, wraw[s, rows, pl.ds(j * 128, 128)], acc)
                    wp[rows, pl.ds(s * D + jp * 128, 128)] = jnp.take_along_axis(acc, src, axis=1)

        qscale = np.float32(DH ** -0.5 * np.log2(np.e))
        masked = np.float32(-1e9 * np.log2(np.e))

        def qkv_sec(i, s):
            x = pltpu.bitcast(ax[pl.ds(i * T2, T2), :], BF16)
            y = jnp.dot(x, pltpu.bitcast(wp[:, s * D:(s + 1) * D], BF16), preferred_element_type=F32)
            if s == 0:
                y = y * qscale
            for j in range(NT):
                qkv[s * NT + j, pl.ds(i * TM + HALO, TM), :] = y[:, j * 128:(j + 1) * 128]

        def attn_steps():
            d1, d2, d3, d4 = dl
            N = (S // RG) * W
            a1, r1, a2, r2, ls, es, acc = {}, {}, {}, {}, {}, {}, {}
            for t in range(N + d1 + d2 + W + d3):
                yield min(S, (t // W + 1) * RG)
                if t < N:
                    g, w = divmod(t, W)
                    r = HALO + g * RG
                    if w == 0:
                        q = [qkv[j, pl.ds(r, RG), :] for j in range(NT)]
                    pr = [q[j] * qkv[NT + j, pl.ds(r - DIL * w, RG), :] for j in range(NT)]
                    a1[t] = tree(add, pr) if qktree else (((pr[0] + pr[1]) + pr[2]) + pr[3]) + pr[4]
                    r1[t] = pltpu.roll(a1[t], 64, 1)
                u = t - d1
                if 0 <= u < N:
                    a2[u] = a1.pop(u) + r1.pop(u)
                    r2[u] = pltpu.roll(a2[u], 32, 1)
                u = t - d1 - d2
                if 0 <= u < N:
                    g, w = divmod(u, W)
                    a = a2.pop(u) + r2.pop(u)
                    if g * RG < DIL * w:
                        pos = lax.broadcasted_iota(I32, (RG, 128), 0) + g * RG
                        a = jnp.where(pos >= DIL * w, a, masked)
                    ls[u] = a
                    if w == W - 1:
                        l8 = [ls.pop(g * W + k) for k in range(W)]
                        m = tree(jnp.maximum, l8)
                        for k in range(W):
                            es[g * W + k] = jnp.exp2(l8[k] - m)
                u = t - d1 - d2 - (W - 1) - d3
                if 0 <= u < N:
                    g, w = divmod(u, W)
                    r = HALO + g * RG
                    if w == 0:
                        den = tree(add, [es[g * W + k] for k in range(W)])
                        inv = pl.reciprocal(den, approx=True)
                    if w == d4 and newton:
                        inv = inv * (2.0 - den * inv)
                    e = es.pop(u)
                    for j in range(NT):
                        p = e * qkv[2 * NT + j, pl.ds(r - DIL * w, RG), :]
                        acc[j] = p if w == 0 else acc[j] + p
                    if w == W - 1:
                        o = [acc[j] * inv for j in range(NT)]
                        if RG >= 16:
                            for j in range(NT):
                                o_s[pl.ds(g * (RG // 2), RG // 2), pl.ds(j * 128, 128)] = pltpu.bitcast(o[j].astype(BF16), I32)
                        elif g % 2 == 0:
                            held = o
                        else:
                            for j in range(NT):
                                o2 = jnp.concatenate([held[j], o[j]], axis=0)
                                o_s[pl.ds((g - 1) * 4, 8), pl.ds(j * 128, 128)] = pltpu.bitcast(o2.astype(BF16), I32)

        wr = jnp.broadcast_to(wr_ref[...].astype(F32).reshape(1, D), (8, D))
        gw = jnp.broadcast_to(gw_ref[...].astype(F32).reshape(1, D), (TM2, D))

        def router(i, racc):
            racc = list(racc)
            for g in range(T2 // 8):
                xw_ = ax[pl.ds(i * T2 + g * 8, 8), :]
                sel = lane == i * (T2 // 8) + g
                for p, xf in enumerate((xw_ << 16, xw_ & HI)):
                    rr = jnp.sum(pltpu.bitcast(xf, F32) * wr, axis=1, keepdims=True)
                    racc[p] = jnp.where(sel, rr, racc[p])
            return tuple(racc)

        def permute_wo():
            for j in range(NT):
                wo_f32[j] = pltpu.bitcast(wo_raw[:, j * 128:(j + 1) * 128], BF16).astype(F32)
            for j in range(NT):
                for d in range(DH):
                    wop[pl.ds(d * 16, 16), pl.ds(j * 128, 128)] = pltpu.bitcast(
                        wo_f32[j, pl.ds(d, 32, stride=DH), :].astype(BF16), I32)

        def ffn(racc):
            sub = lax.broadcasted_iota(I32, (8, 128), 0)
            keys = []
            for p in range(2):
                rr = racc[p].astype(BF16).astype(F32)
                rr = jnp.where(rr == 0, np.float32(0), rr)
                bits = pltpu.bitcast(rr, I32)
                key = jnp.where(bits < 0, bits ^ np.int32(0x7FFF0000), bits)
                key = jnp.where(rr != rr, np.int32(-2**31), key)
                keys.append(key | (S - 1 - (16 * lane + 2 * sub + p)))
            k1 = jnp.max(jnp.maximum(*keys))
            k2 = jnp.max(jnp.maximum(*[jnp.where(k == k1, np.int32(-2**31), k) for k in keys]))
            idx = [S - 1 - (k & (S - 1)) for k in (k1, k2)]
            subD = lax.broadcasted_iota(I32, (16, D), 0)
            sub16 = lax.broadcasted_iota(I32, (16, 128), 0)
            xs, rsel = None, []
            for c, (k, t) in enumerate(zip((k1, k2), idx)):
                blk = pltpu.bitcast(ax[pl.ds(pl.multiple_of((t >> 4) << 3, 8), 8), :], BF16).astype(F32)
                row = jnp.sum(jnp.where(subD == (t & 15), blk, 0.0), axis=0, keepdims=True)
                row = jnp.broadcast_to(row, (16, D))
                xs = row if c == 0 else jnp.where(subD == c, row, xs)
                kb = jnp.full((16, 128), k & HI, I32)
                rsel.append(pltpu.bitcast(jnp.where(kb < 0, kb ^ np.int32(0x7FFF0000), kb), F32))
            xs = xs.astype(BF16)
            dn = (((1,), (1,)), ((), ()))
            gg = lax.dot_general(xs, pltpu.bitcast(wg[...], BF16), dn, preferred_element_type=F32)
            uu = lax.dot_general(xs, pltpu.bitcast(wu[...], BF16), dn, preferred_element_type=F32)
            hh = (jax.nn.silu(gg) * uu).astype(BF16)
            yy = jnp.dot(hh, pltpu.bitcast(wd[...], BF16), preferred_element_type=F32)
            rs = jax.nn.sigmoid(jnp.where(sub16 == 1, rsel[1], rsel[0]))
            yy = yy * jnp.concatenate([rs] * NT, axis=1)
            return idx, yy[0:1], yy[1:2]

        U2 = TM2 // 2

        def out_block(i, idx, y0, y1):
            r0 = i * TM2
            rows = pl.ds(i * U2, U2)
            a = jnp.dot(pltpu.bitcast(o_s[rows, :], BF16), pltpu.bitcast(wop[...], BF16), preferred_element_type=F32)
            b = pltpu.bitcast(ax[rows, :], BF16).astype(F32)
            g = jax.nn.sigmoid(jnp.sum(b * gw, axis=1, keepdims=True))
            pos = lax.broadcasted_iota(I32, (TM2, D), 0)
            b = b + jnp.where(pos == idx[0] - r0, y0, jnp.where(pos == idx[1] - r0, y1, 0.0))
            out_s[rows, :] = pltpu.bitcast((g * a + (1.0 - g) * b).astype(BF16), I32)
            pltpu.make_async_copy(out_s.at[rows], out_h.at[rows], so.at[i]).start()

        for j in range(NT):
            qkv[NT + j, pl.ds(0, HALO), :] = jnp.zeros((HALO, 128), F32)
        for n, s in enumerate(order):
            with scope(f"wait{n}"):
                cp_w[s].wait()
                if n == 0:
                    cp_x[0].wait()
            with scope(f"pro{n}"):
                permute_section(s)
                qkv_sec(0, s)
        for j in range(NT):
            qkv[2 * NT + j, pl.ds(0, HALO), :] = jnp.broadcast_to(qkv[2 * NT + j, pl.ds(HALO, 1), :], (HALO, 128))

        racc = (jnp.zeros((8, 128), F32),) * 2
        att = attn_steps()
        need = next(att)

        def attn_until(rows):
            nonlocal need
            while need is not None and need <= rows:
                need = next(att, None)

        nr = 0
        for i in range(1, NB):
            with scope(f"st{i}"):
                if i in xw:
                    cp_x[1 + xw.index(i)].wait()
                if i == wo_at:
                    cp_wo.wait()
                if i == ffn_at:
                    for c in cp_f:
                        c.wait()
                for s in order:
                    qkv_sec(i, s)
                attn_until(i * TM - (lag * i) // (NB - 1))
                if i in rt:
                    avail = min([b for b in xb if b > i])
                    while nr < min(avail, (rt.index(i) + 1) * NB // len(rt)):
                        racc = router(nr, racc)
                        nr += 1
                if i == wo_at:
                    permute_wo()
                if i == ffn_at:
                    assert nr == NB
                    res = ffn(racc)
        with scope("last"):
            for i in range(nwo):
                out_block(i, *res)
            attn_until(S)
        with scope("ph2"):
            for i in range(nwo, NB2):
                out_block(i, *res)
        with scope("tail"):
            for i in range(NB2):
                pltpu.make_async_copy(out_s.at[pl.ds(i * U2, U2)], out_h.at[pl.ds(i * U2, U2)], so.at[i]).wait()

    def f(A_x, A_wqkv, A_wo, B_x, B_w_r, B_w_gate, B_w_up, B_w_down, gate_w):
        hbm = pl.BlockSpec(memory_space=pltpu.HBM)
        vm = pl.BlockSpec(memory_space=pltpu.VMEM)
        out = pl.pallas_call(
            kern,
            out_shape=jax.ShapeDtypeStruct((S, D), BF16),
            in_specs=[hbm, hbm, hbm, vm, hbm, hbm, hbm, vm],
            out_specs=hbm,
            scratch_shapes=[
                pltpu.VMEM((S // 2, D), I32),
                pltpu.VMEM((3, D // 2, D), I32), pltpu.VMEM((D // 2, 3 * D), I32),
                pltpu.VMEM((D // 2, D), I32), pltpu.VMEM((NT, D, 128), F32), pltpu.VMEM((D // 2, D), I32),
                pltpu.VMEM((F // 2, D), I32), pltpu.VMEM((F // 2, D), I32), pltpu.VMEM((F // 2, D), I32),
                pltpu.VMEM((3 * NT, HALO + S, 128), F32),
                pltpu.VMEM((S // 2, D), I32), pltpu.VMEM((S // 2, D), I32),
                pltpu.SemaphoreType.DMA((len(xw) + 1,)),
                pltpu.SemaphoreType.DMA((7,)), pltpu.SemaphoreType.DMA((NB2,)),
            ],
            compiler_params=pltpu.CompilerParams(vmem_limit_bytes=100 * 2**20, flags=flags),
        )(A_x.reshape(S, D), A_wqkv, A_wo, B_w_r, B_w_gate.T, B_w_up.T, B_w_down, gate_w)
        return out.reshape(1, S, D)
    return f


_impl = make(**dict())


@jax.jit
def pallas_gated_mix__sliding_local_dilated__moe_arch_mod__prompt_kernel(
    A_x, A_wqkv, A_wo, B_x, B_w_r, B_w_gate, B_w_up, B_w_down, gate_w
):
    return _impl(A_x, A_wqkv, A_wo, B_x, B_w_r, B_w_gate, B_w_up, B_w_down, gate_w)
```

```python
import contextlib
import numpy as np
import jax
import jax.numpy as jnp
from jax import lax
from jax.experimental import pallas as pl
from jax.experimental.pallas import tpu as pltpu

S, D, H, DH, W, DIL, F = 2048, 640, 32, 20, 8, 2, 1728
NT = D // 128
HALO = 16
F32, BF16, I32 = jnp.float32, jnp.bfloat16, jnp.int32
HI = np.int32(-65536)


def tree(f, xs):
    while len(xs) > 1:
        xs = [f(xs[k], xs[k + 1]) if k + 1 < len(xs) else xs[k] for k in range(0, len(xs), 2)]
    return xs[0]


def add(a, b):
    return a + b


def plan(att=(256, 512, 768, 1024, 1280, 1536, 1792, 2048), rt=(2, 3, 4), wo=5, ffn=6,
         ob=((256, 256, 256), (256, 256, 256), (256,), (128,), (128,)), wk=(3, 5), ka=384):
    dma = [("w", 1, a, b) for a, b in zip((0,) + wk[:-1], wk)] + [("x", 0, 256), ("x", 256, 512), ("w", 0, 0, 5), ("w", 2, 0, 5),
           ("v",), ("x", 512, S), ("wo",), ("f",)]
    R = [dict(wait=[d], perm=[d[1:]]) for d in dma[:len(wk)]]
    R.append(dict(wait=[("x", 0, 256)], mm=[(1, 0, 256)]))
    R.append(dict(wait=[("x", 256, 512)], mm=[(1, 256, ka - 256)]))
    R.append(dict(wait=[("w", 0, 0, 5)], perm=[(0, 0, 5)], mm=([(1, ka, 512 - ka)] if ka < 512 else []) + [(0, 0, 256)]))
    R.append(dict(wait=[("w", 2, 0, 5)], perm=[(2, 0, 5)], mm=[(0, 256, 256), (2, 0, 256), (2, 256, 256)], halo=True))
    for i in range(2, 8):
        r = dict(mm=[(s, i * 256, 256) for s in (1, 0, 2)], att=att[i - 2], wait=[])
        if i == 2:
            r["wait"] += [("v",), ("x", 512, S)]
        if i in rt:
            k = rt.index(i)
            r["rt"] = (S * k // len(rt) // 16 * 16, S * (k + 1) // len(rt) // 16 * 16)
        if i == wo:
            r["wait"].append(("wo",)); r["wo"] = True
        if i == ffn:
            r["wait"].append(("f",)); r["ffn"] = True
        R.append(r)
    r0 = 0
    for k, blocks in enumerate(ob):
        r = dict(out=[], patch=k == 0)
        for n in blocks:
            r["out"].append((r0, n)); r0 += n
        if 6 + k < len(att):
            r["att"] = att[6 + k]
        R.append(r)
    assert r0 == S
    return dma, R


def make(RG=8, flags=None, scopes=False, dl=(6, 6, 6, 4), qktree=False, newton=True, merge=(), **kw):
    dma, regions = plan(**kw)
    outs = [o for r in regions for o in r.get("out", [])]
    scope = (lambda n: jax.named_scope("Z" + n)) if scopes else (lambda n: contextlib.nullcontext())

    def kern(ax_hbm, wqkv_hbm, wo_hbm, wr_hbm, wg_hbm, wu_hbm, wd_hbm, gw_hbm, out_hbm,
             ax, wraw, wp, wo_raw, wo_f32, wop, wg, wu, wd, qkv, o_s, out_s, g_s, wr_ref, gw_ref, si, so, sbar):
        ax_h, wqkv_h, out_h = (r.bitcast(I32) for r in (ax_hbm, wqkv_hbm, out_hbm))
        cps, nsem = {}, 0
        for d in dma:
            if d[0] == "w":
                rows = pl.ds(d[2] * 64, (d[3] - d[2]) * 64)
                pairs = [(wqkv_h.at[rows, pl.ds(d[1] * D, D)], wraw.at[d[1], rows])]
            elif d[0] == "x":
                rows = pl.ds(d[1] // 2, (d[2] - d[1]) // 2)
                pairs = [(ax_h.at[rows], ax.at[rows])]
            elif d[0] == "v":
                pairs = [(wr_hbm, wr_ref), (gw_hbm, gw_ref)]
            elif d[0] == "wo":
                pairs = [(wo_hbm.bitcast(I32), wo_raw)]
            else:
                pairs = [(h.bitcast(I32), v) for h, v in ((wg_hbm, wg), (wu_hbm, wu), (wd_hbm, wd))]
            cps[d] = [pltpu.make_async_copy(a, b, si.at[nsem + k]) for k, (a, b) in enumerate(pairs)]
            nsem += len(pairs)
            for c in cps[d]:
                c.start()

        lane = lax.broadcasted_iota(I32, (8, 128), 1)

        def permute_chunk(s, k0, k1):
            for jp in range(NT):
                src = (20 * (lane & 31) + 4 * jp + (lane >> 5)) & 127
                tile = (20 * ((13 * ((lane >> 2) - jp)) & 31) + 4 * jp + (lane & 3)) >> 7
                for r in range(k0 * 8, k1 * 8):
                    rows = pl.ds(r * 8, 8)
                    acc = wraw[s, rows, pl.ds(0, 128)]
                    for j in range(1, NT):
                        acc = jnp.where(tile == j, wraw[s, rows, pl.ds(j * 128, 128)], acc)
                    wp[rows, pl.ds(s * D + jp * 128, 128)] = jnp.take_along_axis(acc, src, axis=1)

        qscale = np.float32(DH ** -0.5 * np.log2(np.e))
        masked = np.float32(-1e9 * np.log2(np.e))

        def qkv_mm(s, r0, n):
            x = pltpu.bitcast(ax[pl.ds(r0 // 2, n // 2), :], BF16)
            y = jnp.dot(x, pltpu.bitcast(wp[:, s * D:(s + 1) * D], BF16), preferred_element_type=F32)
            if s == 0:
                y = y * qscale
            for j in range(NT):
                qkv[s * NT + j, pl.ds(r0 + HALO, n), :] = y[:, j * 128:(j + 1) * 128]

        def attn_steps():
            d1, d2, d3, d4 = dl
            N = (S // RG) * W
            a1, r1, a2, r2, ls, es, acc = {}, {}, {}, {}, {}, {}, {}
            for t in range(N + d1 + d2 + W + d3):
                yield min(S, (t // W + 1) * RG)
                if t < N:
                    g, w = divmod(t, W)
                    r = HALO + g * RG
                    if w == 0:
                        q = [qkv[j, pl.ds(r, RG), :] for j in range(NT)]
                    pr = [q[j] * qkv[NT + j, pl.ds(r - DIL * w, RG), :] for j in range(NT)]
                    a1[t] = tree(add, pr) if qktree else (((pr[0] + pr[1]) + pr[2]) + pr[3]) + pr[4]
                    r1[t] = pltpu.roll(a1[t], 64, 1)
                u = t - d1
                if 0 <= u < N:
                    a2[u] = a1.pop(u) + r1.pop(u)
                    r2[u] = pltpu.roll(a2[u], 32, 1)
                u = t - d1 - d2
                if 0 <= u < N:
                    g, w = divmod(u, W)
                    a = a2.pop(u) + r2.pop(u)
                    if g * RG < DIL * w:
                        pos = lax.broadcasted_iota(I32, (RG, 128), 0) + g * RG
                        a = jnp.where(pos >= DIL * w, a, masked)
                    ls[u] = a
                    if w == W - 1:
                        l8 = [ls.pop(g * W + k) for k in range(W)]
                        m = tree(jnp.maximum, l8)
                        for k in range(W):
                            es[g * W + k] = jnp.exp2(l8[k] - m)
                u = t - d1 - d2 - (W - 1) - d3
                if 0 <= u < N:
                    g, w = divmod(u, W)
                    r = HALO + g * RG
                    if w == 0:
                        den = tree(add, [es[g * W + k] for k in range(W)])
                        inv = pl.reciprocal(den, approx=True)
                    if w == d4 and newton:
                        inv = inv * (2.0 - den * inv)
                    e = es.pop(u)
                    for j in range(NT):
                        p = e * qkv[2 * NT + j, pl.ds(r - DIL * w, RG), :]
                        acc[j] = p if w == 0 else acc[j] + p
                    if w == W - 1:
                        o = [acc[j] * inv for j in range(NT)]
                        if RG >= 16:
                            for j in range(NT):
                                o_s[pl.ds(g * (RG // 2), RG // 2), pl.ds(j * 128, 128)] = pltpu.bitcast(o[j].astype(BF16), I32)
                        elif g % 2 == 0:
                            held = o
                        else:
                            for j in range(NT):
                                o2 = jnp.concatenate([held[j], o[j]], axis=0)
                                o_s[pl.ds((g - 1) * 4, 8), pl.ds(j * 128, 128)] = pltpu.bitcast(o2.astype(BF16), I32)

        def router(ra, rb, racc):
            racc = list(racc)
            wr = jnp.broadcast_to(wr_ref[...].astype(F32).reshape(1, D), (8, D))
            gw = jnp.broadcast_to(gw_ref[...].astype(F32).reshape(1, D), (8, D))
            for g in range(ra // 16, rb // 16):
                xf = pltpu.bitcast(ax[pl.ds(g * 8, 8), :], BF16).astype(F32)
                for p in range(2):
                    n = 2 * g + p
                    xp = xf[8 * p:8 * p + 8]
                    rr = jnp.sum(xp * wr, axis=1, keepdims=True)
                    racc[n // 128] = jnp.where(lane == n % 128, rr, racc[n // 128])
                    g_s[pl.ds(n * 8, 8), :] = jnp.broadcast_to(jnp.sum(xp * gw, axis=1, keepdims=True), (8, 128))
            return tuple(racc)

        def permute_wo():
            for j in range(NT):
                wo_f32[j] = pltpu.bitcast(wo_raw[:, j * 128:(j + 1) * 128], BF16).astype(F32)
            for j in range(NT):
                for d in range(DH):
                    wop[pl.ds(d * 16, 16), pl.ds(j * 128, 128)] = pltpu.bitcast(
                        wo_f32[j, pl.ds(d, 32, stride=DH), :].astype(BF16), I32)

        def ffn(racc):
            sub = lax.broadcasted_iota(I32, (8, 128), 0)
            keys = []
            for p in range(2):
                rr = racc[p].astype(BF16).astype(F32)
                rr = jnp.where(rr == 0, np.float32(0), rr)
                bits = pltpu.bitcast(rr, I32)
                key = jnp.where(bits < 0, bits ^ np.int32(0x7FFF0000), bits)
                key = jnp.where(rr != rr, np.int32(-2**31), key)
                keys.append(key | (S - 1 - (1024 * p + 8 * lane + sub)))
            k1 = jnp.max(jnp.maximum(*keys))
            k2 = jnp.max(jnp.maximum(*[jnp.where(k == k1, np.int32(-2**31), k) for k in keys]))
            idx = [S - 1 - (k & (S - 1)) for k in (k1, k2)]
            subD = lax.broadcasted_iota(I32, (16, D), 0)
            sub16 = lax.broadcasted_iota(I32, (16, 128), 0)
            xs, rsel = None, []
            for c, (k, t) in enumerate(zip((k1, k2), idx)):
                blk = pltpu.bitcast(ax[pl.ds(pl.multiple_of((t >> 4) << 3, 8), 8), :], BF16).astype(F32)
                row = jnp.sum(jnp.where(subD == (t & 15), blk, 0.0), axis=0, keepdims=True)
                row = jnp.broadcast_to(row, (16, D))
                xs = row if c == 0 else jnp.where(subD == c, row, xs)
                kb = jnp.full((16, 128), k & HI, I32)
                rsel.append(pltpu.bitcast(jnp.where(kb < 0, kb ^ np.int32(0x7FFF0000), kb), F32))
            xs = xs.astype(BF16)
            dn = (((1,), (1,)), ((), ()))
            gg = lax.dot_general(xs, pltpu.bitcast(wg[...], BF16), dn, preferred_element_type=F32)
            uu = lax.dot_general(xs, pltpu.bitcast(wu[...], BF16), dn, preferred_element_type=F32)
            hh = (jax.nn.silu(gg) * uu).astype(BF16)
            yy = jnp.dot(hh, pltpu.bitcast(wd[...], BF16), preferred_element_type=F32)
            rs = jax.nn.sigmoid(jnp.where(sub16 == 1, rsel[1], rsel[0]))
            yy = yy * jnp.concatenate([rs] * NT, axis=1)
            return idx, yy

        def patch(idx, yy):
            subD = lax.broadcasted_iota(I32, (16, D), 0)
            for c, t in enumerate(idx):
                rows = pl.ds(pl.multiple_of((t >> 4) << 3, 8), 8)
                blk = pltpu.bitcast(ax[rows, :], BF16).astype(F32)
                blk = jnp.where(subD == (t & 15), blk + yy[c:c + 1], blk)
                ax[rows, :] = pltpu.bitcast(blk.astype(BF16), I32)

        cp_o = [pltpu.make_async_copy(out_s.at[pl.ds(r0 // 2, n // 2)], out_h.at[pl.ds(r0 // 2, n // 2)], so.at[i])
                for i, (r0, n) in enumerate(outs)]

        def out_block(r0, n):
            rows = pl.ds(r0 // 2, n // 2)
            a = jnp.dot(pltpu.bitcast(o_s[rows, :], BF16), pltpu.bitcast(wop[...], BF16), preferred_element_type=F32)
            b = pltpu.bitcast(ax[rows, :], BF16).astype(F32)
            g = jax.nn.sigmoid(g_s[pl.ds(r0, n), :])
            g = jnp.concatenate([g] * NT, axis=1)
            out_s[rows, :] = pltpu.bitcast((b + g * (a - b)).astype(BF16), I32)

        for j in range(NT):
            qkv[NT + j, pl.ds(0, HALO), :] = jnp.zeros((HALO, 128), F32)
        racc = (jnp.zeros((8, 128), F32),) * 2
        att = attn_steps()
        need = next(att)
        for k, r in enumerate(regions):
            with scope(str(k)):
                for d in r.get("wait", []):
                    for c in cps[d]:
                        c.wait()
                if k not in merge:
                    pl.semaphore_signal(sbar, 1)
                    pl.semaphore_wait(sbar, 1)
                if r.get("patch"):
                    patch(*res)
                for p in r.get("perm", []):
                    permute_chunk(*p)
                for m in r.get("mm", []):
                    qkv_mm(*m)
                if r.get("halo"):
                    for j in range(NT):
                        qkv[2 * NT + j, pl.ds(0, HALO), :] = jnp.broadcast_to(qkv[2 * NT + j, pl.ds(HALO, 1), :], (HALO, 128))
                for o in r.get("out", []):
                    out_block(*o)
                while need is not None and need <= r.get("att", 0):
                    need = next(att, None)
                if "rt" in r:
                    racc = router(*r["rt"], racc)
                if r.get("wo"):
                    permute_wo()
                if r.get("ffn"):
                    res = ffn(racc)
                for o in r.get("out", []):
                    cp_o[outs.index(o)].start()
        with scope("tail"):
            for c in cp_o:
                c.wait()

    def f(A_x, A_wqkv, A_wo, B_x, B_w_r, B_w_gate, B_w_up, B_w_down, gate_w):
        hbm = pl.BlockSpec(memory_space=pltpu.HBM)
        vm = pl.BlockSpec(memory_space=pltpu.VMEM)
        out = pl.pallas_call(
            kern,
            out_shape=jax.ShapeDtypeStruct((S, D), BF16),
            in_specs=[hbm] * 8,
            out_specs=hbm,
            scratch_shapes=[
                pltpu.VMEM((S // 2, D), I32),
                pltpu.VMEM((3, D // 2, D), I32), pltpu.VMEM((D // 2, 3 * D), I32),
                pltpu.VMEM((D // 2, D), I32), pltpu.VMEM((NT, D, 128), F32), pltpu.VMEM((D // 2, D), I32),
                pltpu.VMEM((F // 2, D), I32), pltpu.VMEM((F // 2, D), I32), pltpu.VMEM((F // 2, D), I32),
                pltpu.VMEM((3 * NT, HALO + S, 128), F32),
                pltpu.VMEM((S // 2, D), I32), pltpu.VMEM((S // 2, D), I32),
                pltpu.VMEM((S, 128), F32), pltpu.VMEM((D,), BF16), pltpu.VMEM((D,), BF16),
                pltpu.SemaphoreType.DMA((len(dma) + 3,)), pltpu.SemaphoreType.DMA((len(outs),)), pltpu.SemaphoreType.REGULAR,
            ],
            compiler_params=pltpu.CompilerParams(vmem_limit_bytes=100 * 2**20, flags=flags),
        )(A_x.reshape(S, D), A_wqkv, A_wo, B_w_r, B_w_gate.T, B_w_up.T, B_w_down, gate_w)
        return out.reshape(1, S, D)
    return f


_impl = make(**dict(merge=(6, 8, 11)))


@jax.jit
def pallas_gated_mix__sliding_local_dilated__moe_arch_mod__prompt_kernel(
    A_x, A_wqkv, A_wo, B_x, B_w_r, B_w_gate, B_w_up, B_w_down, gate_w
):
    return _impl(A_x, A_wqkv, A_wo, B_x, B_w_r, B_w_gate, B_w_up, B_w_down, gate_w)
```

```python
import contextlib
import numpy as np
import jax
import jax.numpy as jnp
from jax import lax
from jax.experimental import pallas as pl
from jax.experimental.pallas import tpu as pltpu

S, D, H, DH, W, DIL, F = 2048, 640, 32, 20, 8, 2, 1728
NT = D // 128
HALO = 16
PITCH = 20
F32, BF16, I32 = jnp.float32, jnp.bfloat16, jnp.int32
HI = np.int32(-65536)


def tree(f, xs):
    while len(xs) > 1:
        xs = [f(xs[k], xs[k + 1]) if k + 1 < len(xs) else xs[k] for k in range(0, len(xs), 2)]
    return xs[0]


def add(a, b):
    return a + b


def plan(att=(256, 512, 768, 1024, 1280, 1568, 1816, 2048), rt={2: 1024, 3: 2048}, wo={4: (0, 1, 2, 3, 4)}, wow=4, fatt=1600, sel_at=4, ffn=7, xp={5: (0, 40), 6: (40, 80), 7: (80, 108)},
         ob=((256, 256, 256), (256, 256, 256), (256,), (128,), (128,)), wk=(3, 5), ka=384, st=(256,) * 6, v5=256):
    dma = [("w", 1, a, b) for a, b in zip((0,) + wk[:-1], wk)] + [("x", 0, 256), ("x", 256, 512), ("w", 0, 0, 5), ("w", 2, 0, 5),
           ("v",)] + [("x", 512, S)] + [("wo",), ("f",)]
    R = [dict(wait=[d], perm=[d[1:]]) for d in dma[:len(wk)]]
    R.append(dict(wait=[("x", 0, 256)], mm=[(1, 0, 256)]))
    R.append(dict(wait=[("x", 256, 512)], mm=[(1, 256, ka - 256)]))
    R.append(dict(wait=[("w", 0, 0, 5)], perm=[(0, 0, 5)], mm=([(1, ka, 512 - ka)] if ka < 512 else []) + [(0, 0, 256)]))
    R.append(dict(wait=[("w", 2, 0, 5)], perm=[(2, 0, 5)], mm=[(0, 256, 256)] + [(2, a, v5) for a in range(0, 512, v5)], halo=True))
    q0, n_st, nr = 512, len(st), 0
    assert q0 + sum(st) == S
    for i in range(2, 2 + n_st):
        r = dict(mm=[(s, q0, st[i - 2]) for s in (1, 0, 2)], att=att[i - 2], wait=[])
        q0 += st[i - 2]
        if i == 2:
            r["wait"] += [("v",), ("x", 512, S)]
        if i in rt:
            r["rt"] = (nr, rt[i]); nr = rt[i]
        if i in wo:
            r["wo"] = wo[i]
        if i == wow:
            r["wait"].append(("wo",))
        if i == sel_at:
            r["select"] = True
        if i in xp:
            r["xp"] = range(*xp[i])
        if i == (min(xp) if xp else ffn):
            r["wait"].append(("f",))
        if i == ffn:
            r["ffn"] = True
        R.append(r)
    r0 = 0
    for k, blocks in enumerate(ob):
        if k == 0 and ffn == 0:
            R.append(dict(wait=[] if xp else [("f",)], ffn=True, att=fatt))
            if not wo:
                R[-1]["wait"].append(("wo",)); R[-1]["wo"] = tuple(range(NT))
        r = dict(out=[], patch=k == 0)
        for n in blocks:
            r["out"].append((r0, n)); r0 += n
        if n_st + k < len(att):
            r["att"] = att[n_st + k]
        R.append(r)
    assert r0 == S
    return dma, R


def make(RG=8, flags=None, scopes=False, dl=(6, 6, 6, 4), qktree=False, newton=True, merge=(), defer=0, ring=S, auxpos="start", **kw):
    dma, regions = plan(**kw)
    outs = [o for r in regions for o in r.get("out", [])]
    scope = (lambda n: jax.named_scope("Z" + n)) if scopes else (lambda n: contextlib.nullcontext())

    def kern(ax_hbm, wqkv_hbm, wo_hbm, wr_hbm, wg_hbm, wu_hbm, wd_hbm, gw_hbm, out_hbm,
             ax, wraw, wp, wo_raw, wop, wg, wu, wd, xsel, hbuf, qkv, o_s, out_s, g_s, wr_ref, gw_ref, si, so, sbar):
        ax_h, wqkv_h, out_h = (r.bitcast(I32) for r in (ax_hbm, wqkv_hbm, out_hbm))
        cps, nsem = {}, 0
        for d in dma:
            if d[0] == "w":
                rows = pl.ds(d[2] * 64, (d[3] - d[2]) * 64)
                pairs = [(wqkv_h.at[rows, pl.ds(d[1] * D, D)], wraw.at[d[1], rows])]
            elif d[0] == "x":
                rows = pl.ds(d[1] // 2, (d[2] - d[1]) // 2)
                pairs = [(ax_h.at[rows], ax.at[rows])]
            elif d[0] == "v":
                pairs = [(wr_hbm, wr_ref), (gw_hbm, gw_ref)]
            elif d[0] == "wo":
                pairs = [(wo_hbm.bitcast(I32).at[:, pl.ds(j * 128, 128)], wo_raw.at[j]) for j in range(NT)]
            else:
                pairs = [(h.bitcast(I32), v) for h, v in ((wg_hbm, wg), (wu_hbm, wu), (wd_hbm, wd))]
            cps[d] = [pltpu.make_async_copy(a, b, si.at[nsem + k]) for k, (a, b) in enumerate(pairs)]
            nsem += len(pairs)
            for c in cps[d]:
                c.start()

        lane = lax.broadcasted_iota(I32, (8, 128), 1)

        def permute_chunk(s, k0, k1):
            for jp in range(NT):
                src = (20 * (lane & 31) + 4 * jp + (lane >> 5)) & 127
                tile = (20 * ((13 * ((lane >> 2) - jp)) & 31) + 4 * jp + (lane & 3)) >> 7
                for r in range(k0 * 8, k1 * 8):
                    rows = pl.ds(r * 8, 8)
                    acc = wraw[s, rows, pl.ds(0, 128)]
                    for j in range(1, NT):
                        acc = jnp.where(tile == j, wraw[s, rows, pl.ds(j * 128, 128)], acc)
                    wp[rows, pl.ds(s * D + jp * 128, 128)] = jnp.take_along_axis(acc, src, axis=1)

        qscale = np.float32(DH ** -0.5 * np.log2(np.e))
        masked = np.float32(-1e9 * np.log2(np.e))

        def qkv_mm(s, r0, n):
            x = pltpu.bitcast(ax[pl.ds(r0 // 2, n // 2), :], BF16)
            y = jnp.dot(x, pltpu.bitcast(wp[:, s * D:(s + 1) * D], BF16), preferred_element_type=F32)
            if s == 0:
                y = y * qscale

            def store():
                p0 = r0 % ring
                for j in range(NT):
                    qkv[s * NT + j, pl.ds(p0 + HALO, n), :] = y[:, j * 128:(j + 1) * 128]
                    if s > 0 and p0 + n == ring and r0 + n < S:
                        qkv[s * NT + j, pl.ds(0, HALO), :] = y[n - HALO:, j * 128:(j + 1) * 128]
            return store

        att_done = 0

        def attn_steps():
            d1, d2, d3, d4 = dl
            N = (S // RG) * W
            nonlocal att_done
            a1, r1, a2, r2, ls, es, acc = {}, {}, {}, {}, {}, {}, {}
            for t in range(N + d1 + d2 + W + d3):
                yield min(S, (t // W + 1) * RG)
                if t < N:
                    g, w = divmod(t, W)
                    r = HALO + (g * RG) % ring
                    if w == 0:
                        q = [qkv[j, pl.ds(r, RG), :] for j in range(NT)]
                    pr = [q[j] * qkv[NT + j, pl.ds(r - DIL * w, RG), :] for j in range(NT)]
                    a1[t] = tree(add, pr) if qktree else (((pr[0] + pr[1]) + pr[2]) + pr[3]) + pr[4]
                    r1[t] = pltpu.roll(a1[t], 64, 1)
                u = t - d1
                if 0 <= u < N:
                    a2[u] = a1.pop(u) + r1.pop(u)
                    r2[u] = pltpu.roll(a2[u], 32, 1)
                u = t - d1 - d2
                if 0 <= u < N:
                    g, w = divmod(u, W)
                    a = a2.pop(u) + r2.pop(u)
                    if g * RG < DIL * w:
                        pos = lax.broadcasted_iota(I32, (RG, 128), 0) + g * RG
                        a = jnp.where(pos >= DIL * w, a, masked)
                    ls[u] = a
                    if w == W - 1:
                        l8 = [ls.pop(g * W + k) for k in range(W)]
                        m = tree(jnp.maximum, l8)
                        for k in range(W):
                            es[g * W + k] = jnp.exp2(l8[k] - m)
                u = t - d1 - d2 - (W - 1) - d3
                if 0 <= u < N:
                    g, w = divmod(u, W)
                    r = HALO + (g * RG) % ring
                    if w == 0:
                        den = tree(add, [es[g * W + k] for k in range(W)])
                        inv = pl.reciprocal(den, approx=True)
                    if w == d4 and newton:
                        inv = inv * (2.0 - den * inv)
                    e = es.pop(u)
                    for j in range(NT):
                        p = e * qkv[2 * NT + j, pl.ds(r - DIL * w, RG), :]
                        acc[j] = p if w == 0 else acc[j] + p
                    if w == W - 1:
                        o = [acc[j] * inv for j in range(NT)]
                        if RG >= 16:
                            for j in range(NT):
                                o_s[pl.ds(g * (RG // 2), RG // 2), pl.ds(j * 128, 128)] = pltpu.bitcast(o[j].astype(BF16), I32)
                        elif g % 2 == 0:
                            held = o
                        else:
                            for j in range(NT):
                                o2 = jnp.concatenate([held[j], o[j]], axis=0)
                                o_s[pl.ds((g - 1) * 4, 8), pl.ds(j * 128, 128)] = pltpu.bitcast(o2.astype(BF16), I32)
                            att_done = (g + 1) * RG

        racc = [jnp.zeros((8, 128), F32)] * 2
        vecs = []

        def router(g):
            if not vecs:
                vecs.extend(jnp.broadcast_to(v[...].astype(F32).reshape(1, D), (8, D)) for v in (wr_ref, gw_ref))
            xf = pltpu.bitcast(ax[pl.ds(g * 8, 8), :], BF16).astype(F32)
            for p in range(2):
                n = 2 * g + p
                xp = xf[8 * p:8 * p + 8]
                rr = jnp.sum(xp * vecs[0], axis=1, keepdims=True)
                racc[n // 128] = jnp.where(lane == n % 128, rr, racc[n // 128])
                g_s[pl.ds(n * 8, 8), :] = jnp.broadcast_to(jnp.sum(xp * vecs[1], axis=1, keepdims=True), (8, 128))

        def wo_gather(j, d2):
            ev = wo_raw[j, pl.ds(d2, H // 2, stride=DH), :]
            od = wo_raw[j, pl.ds(DH // 2 + d2, H // 2, stride=DH), :]
            cols = pl.ds(j * 128, 128)
            wop[pl.ds(d2 * 32, 16), cols] = (ev & 0xFFFF) | (od << 16)
            wop[pl.ds(d2 * 32 + 16, 16), cols] = lax.shift_right_logical(ev, 16) | (od & HI)

        sub = lax.broadcasted_iota(I32, (8, 128), 0)
        sel = {}

        def select():
            keys = []
            for p in range(2):
                rr = racc[p].astype(BF16).astype(F32)
                rr = jnp.where(rr == 0, np.float32(0), rr)
                bits = pltpu.bitcast(rr, I32)
                key = jnp.where(bits < 0, bits ^ np.int32(0x7FFF0000), bits)
                key = jnp.where(rr != rr, np.int32(-2**31), key)
                keys.append(key | (S - 1 - (1024 * p + 8 * lane + sub)))
            k1 = jnp.max(jnp.maximum(*keys))
            k2 = jnp.max(jnp.maximum(*[jnp.where(k == k1, np.int32(-2**31), k) for k in keys]))
            sel["idx"] = [S - 1 - (k & (S - 1)) for k in (k1, k2)]
            sel["keys"] = (k1, k2)
            subD = lax.broadcasted_iota(I32, (16, D), 0)
            for c, t in enumerate(sel["idx"]):
                blk = pltpu.bitcast(ax[pl.ds(pl.multiple_of((t >> 4) << 3, 8), 8), :], BF16).astype(F32)
                row = jnp.sum(jnp.where(subD == (t & 15), blk, 0.0), axis=0, keepdims=True)
                xsel[c] = jnp.broadcast_to(row, (8, D))

        pre = {}

        def gate_up(l):
            T = l // 8
            for m, w_ref in enumerate((wg, wu)):
                ww = w_ref[pl.ds(l * 8, 8), :]
                for p, wf in enumerate((ww << 16, ww & HI)):
                    wf = pltpu.bitcast(wf, F32)
                    here = lane - 2 * sub == 16 * (l % 8) + p
                    for c in range(2):
                        val = jnp.sum(wf * xsel[c], axis=1, keepdims=True)
                        pre[m, c] = jnp.where(here, val, pre.get((m, c), np.float32(0)))
            if l % 8 == 7 or l == F // 16 - 1:
                hh = jnp.concatenate([jax.nn.silu(pre.pop((0, c))) * pre.pop((1, c)) for c in range(2)], axis=0)
                hbuf[:, pl.ds(T * 128, 128)] = pltpu.bitcast(hh.astype(BF16), I32)

        def down():
            yy = jnp.dot(pltpu.bitcast(hbuf[:, pl.ds(0, F)], BF16), pltpu.bitcast(wd[...], BF16), preferred_element_type=F32)
            ys = []
            for c, k in enumerate(sel["keys"]):
                kb = jnp.full((1, 128), k & HI, I32)
                rs = jax.nn.sigmoid(pltpu.bitcast(jnp.where(kb < 0, kb ^ np.int32(0x7FFF0000), kb), F32))
                ys.append(jnp.sum(yy[8 * c:8 * c + 8], axis=0, keepdims=True) * jnp.concatenate([rs] * NT, axis=1))
            return sel["idx"], ys

        def patch(idx, yy):
            subD = lax.broadcasted_iota(I32, (16, D), 0)
            for c, t in enumerate(idx):
                rows = pl.ds(pl.multiple_of((t >> 4) << 3, 8), 8)
                blk = pltpu.bitcast(ax[rows, :], BF16).astype(F32)
                blk = jnp.where(subD == (t & 15), blk + yy[c], blk)
                ax[rows, :] = pltpu.bitcast(blk.astype(BF16), I32)

        cp_o = [pltpu.make_async_copy(out_s.at[pl.ds(r0 // 2, n // 2)], out_h.at[pl.ds(r0 // 2, n // 2)], so.at[i])
                for i, (r0, n) in enumerate(outs)]

        def out_block(r0, n):
            assert att_done >= r0 + n
            rows = pl.ds(r0 // 2, n // 2)
            a = jnp.dot(pltpu.bitcast(o_s[rows, :], BF16), pltpu.bitcast(wop[...], BF16), preferred_element_type=F32)
            b = pltpu.bitcast(ax[rows, :], BF16).astype(F32)
            g = jax.nn.sigmoid(g_s[pl.ds(r0, n), :])
            g = jnp.concatenate([g] * NT, axis=1)
            out_s[rows, :] = pltpu.bitcast((b + g * (a - b)).astype(BF16), I32)

        for j in range(NT):
            qkv[NT + j, pl.ds(0, HALO), :] = jnp.zeros((HALO, 128), F32)
        att = attn_steps()
        need = next(att)
        pending = []

        def run_aux(r):
            if "rt" in r:
                for g in range(r["rt"][0] // 16, r["rt"][1] // 16):
                    router(g)
            if r.get("select"):
                select()
            for l in r.get("xp", ()):
                gate_up(l)
            for j in r.get("wo", ()):
                for d in range(DH // 2):
                    wo_gather(j, d)

        for k, r in enumerate(regions):
            with scope(str(k)):
                for d in r.get("wait", []):
                    for c in cps[d]:
                        c.wait()
                if k not in merge:
                    pl.semaphore_signal(sbar, 1)
                    pl.semaphore_wait(sbar, 1)
                if r.get("patch"):
                    patch(*res)
                for p in r.get("perm", []):
                    permute_chunk(*p)
                for fn in pending:
                    fn()
                pending = []
                if auxpos == "start":
                    run_aux(r)
                mms = list(r.get("mm", []))
                if defer and mms and k + 1 < len(regions) and not r.get("halo"):
                    s_, r0, n = mms.pop()
                    if n > defer:
                        mms.append((s_, r0, n - defer))
                    for m in mms:
                        qkv_mm(*m)()
                    pending.append(qkv_mm(s_, r0 + n - min(n, defer), min(n, defer)))
                else:
                    for m in mms:
                        qkv_mm(*m)()
                if r.get("halo"):
                    for j in range(NT):
                        qkv[2 * NT + j, pl.ds(0, HALO), :] = jnp.broadcast_to(qkv[2 * NT + j, pl.ds(HALO, 1), :], (HALO, 128))
                late = [o for o in r.get("out", []) if att_done < sum(o)]
                for o in r.get("out", []):
                    if o not in late:
                        out_block(*o)
                if auxpos == "mid":
                    run_aux(r)
                while need is not None and need <= r.get("att", 0):
                    need = next(att, None)
                for o in late:
                    out_block(*o)
                if auxpos == "end":
                    run_aux(r)
                if r.get("ffn"):
                    res = down()
                for o in r.get("out", []):
                    cp_o[outs.index(o)].start()
        with scope("tail"):
            for c in cp_o:
                c.wait()

    def f(A_x, A_wqkv, A_wo, B_x, B_w_r, B_w_gate, B_w_up, B_w_down, gate_w):
        hbm = pl.BlockSpec(memory_space=pltpu.HBM)
        vm = pl.BlockSpec(memory_space=pltpu.VMEM)
        out = pl.pallas_call(
            kern,
            out_shape=jax.ShapeDtypeStruct((S, D), BF16),
            in_specs=[hbm] * 8,
            out_specs=hbm,
            scratch_shapes=[
                pltpu.VMEM((S // 2, D), I32),
                pltpu.VMEM((3, D // 2, D), I32), pltpu.VMEM((D // 2, 3 * D), I32),
                pltpu.VMEM((NT, D // 2, 128), I32), pltpu.VMEM((D // 2, D), I32),
                pltpu.VMEM((F // 2, D), I32), pltpu.VMEM((F // 2, D), I32), pltpu.VMEM((F // 2, D), I32),
                pltpu.VMEM((2, 8, D), F32), pltpu.VMEM((8, 1792), I32),
                pltpu.VMEM((3 * NT, HALO + ring, 128), F32),
                pltpu.VMEM((S // 2, D), I32), pltpu.VMEM((S // 2, D), I32),
                pltpu.VMEM((S, 128), F32), pltpu.VMEM((D,), BF16), pltpu.VMEM((D,), BF16),
                pltpu.SemaphoreType.DMA((len(dma) + 7,)), pltpu.SemaphoreType.DMA((len(outs),)), pltpu.SemaphoreType.REGULAR,
            ],
            compiler_params=pltpu.CompilerParams(vmem_limit_bytes=100 * 2**20, flags=flags),
        )(A_x.reshape(S, D), A_wqkv, A_wo, B_w_r, B_w_gate.T, B_w_up.T, B_w_down, gate_w)
        return out.reshape(1, S, D)
    return f


_impl = make(**dict(ob=((256,)*3,(256,)*3,(384,),(128,))))


@jax.jit
def pallas_gated_mix__sliding_local_dilated__moe_arch_mod__prompt_kernel(
    A_x, A_wqkv, A_wo, B_x, B_w_r, B_w_gate, B_w_up, B_w_down, gate_w
):
    return _impl(A_x, A_wqkv, A_wo, B_x, B_w_r, B_w_gate, B_w_up, B_w_down, gate_w)
```

```python
import contextlib
import numpy as np
import jax
import jax.numpy as jnp
from jax import lax
from jax.experimental import pallas as pl
from jax.experimental.pallas import tpu as pltpu

S, D, H, DH, W, DIL, F = 2048, 640, 32, 20, 8, 2, 1728
NT = D // 128
HALO = 16
PITCH = 20
F32, BF16, I32 = jnp.float32, jnp.bfloat16, jnp.int32
HI = np.int32(-65536)


def tree(f, xs):
    while len(xs) > 1:
        xs = [f(xs[k], xs[k + 1]) if k + 1 < len(xs) else xs[k] for k in range(0, len(xs), 2)]
    return xs[0]


def add(a, b):
    return a + b


def plan(att=(0, 256, 512, 768, 1024, 1280, 1536, 1792, 2048), x2=768, rt=(1408, 2048), wo=3, sel_at=3,
         xp={4: (0, 40), 5: (40, 80), 6: (80, 108)}, ffn=6, kc=2, wk=(3, 5),
         ob=((256, 256, 256), (256, 256, 256), (384,), (128,))):
    if kc:
        dma = [("xc", 0, kc), ("w", 1, 0, kc), ("xc", kc, 5), ("w", 1, kc, 5)]
        R = [dict(wait=dma[:2], perm=[(1, 0, kc)], kmm=(0, kc)), dict(wait=dma[2:], perm=[(1, kc, 5)], kmm=(kc, 5))]
        R.append(dict(wait=[("w", 0, 0, 5)], perm=[(0, 0, 5)], mm=[(0, 0, 256)]))
    else:
        dma = [("w", 1, a, b) for a, b in zip((0,) + wk[:-1], wk)] + [("x", 0, 256), ("x", 256, 512)]
        R = [dict(wait=[d], perm=[d[1:]]) for d in dma[:len(wk)]]
        R.append(dict(wait=[("x", 0, 256)], mm=[(1, 0, 256)]))
        R.append(dict(wait=[("x", 256, 512)], mm=[(1, 256, 128)]))
        R.append(dict(wait=[("w", 0, 0, 5)], perm=[(0, 0, 5)], mm=[(1, 384, 128), (0, 0, 256)]))
    dma += [("w", 0, 0, 5), ("w", 2, 0, 5), ("v",), ("x", 512, x2), ("x", x2, S), ("wo",), ("f",), ("d",)]
    R.append(dict(wait=[("w", 2, 0, 5), ("v",), ("x", 512, x2)], perm=[(2, 0, 5)], halo=True, rt=(0, x2), att=att[0],
                  mm=[(2, 0, 256), (0, 256, 256), (2, 256, 256)], name=0))
    nr = x2
    for i in range(1, 7):
        r = dict(mm=[(s, 256 + 256 * i, 256) for s in (1, 0, 2)], att=att[i], wait=[], name=i)
        if i == 1:
            r["wait"] += [("x", x2, S), ("wo",)]
        if i <= len(rt):
            r["rt"] = (nr, rt[i - 1]); nr = rt[i - 1]
        if i == wo:
            r["wo"] = range(NT)
        if i == sel_at:
            r["select"] = True
        if i in xp:
            r["xp"] = range(*xp[i])
        if i == min(xp):
            r["wait"] += [("f",), ("d",)]
        if i == ffn:
            r["ffn"] = True
        R.append(r)
    r0 = 0
    for k, blocks in enumerate(ob):
        r = dict(out=[], patch=k == 0, name=7 + k)
        for n in blocks:
            r["out"].append((r0, n)); r0 += n
        if 7 + k < len(att):
            r["att"] = att[7 + k]
        R.append(r)
    for a, b in zip(R[:-1], R[1:]):
        if "out" in b:
            a["gx"] = (b["out"][0][0], sum(b["out"][-1]))
    assert r0 == S and nr == S
    return dma, R


def make(RG=8, flags=None, scopes=False, dl=(6, 6, 6, 4), qktree=False, newton=True, merge=(), defer=0, ring=S, auxpos="start", **kw):
    dma, regions = plan(**kw)
    outs = [o for r in regions for o in r.get("out", [])]
    scope = (lambda n: jax.named_scope("Z" + n)) if scopes else (lambda n: contextlib.nullcontext())

    def kern(ax_hbm, wqkv_hbm, wo_hbm, wr_hbm, wg_hbm, wu_hbm, wd_hbm, gw_hbm, out_hbm,
             ax, wraw, wp, wo_raw, wop, wg, wu, wd, xsel, hbuf, qkv, o_s, out_s, g_s, g_rep, wr_ref, gw_ref, si, so, sbar):
        ax_h, wqkv_h, out_h = (r.bitcast(I32) for r in (ax_hbm, wqkv_hbm, out_hbm))
        cps, nsem = {}, 0
        for d in dma:
            if d[0] == "w":
                rows = pl.ds(d[2] * 64, (d[3] - d[2]) * 64)
                pairs = [(wqkv_h.at[rows, pl.ds(d[1] * D, D)], wraw.at[d[1], rows])]
            elif d[0] == "x":
                rows = pl.ds(d[1] // 2, (d[2] - d[1]) // 2)
                pairs = [(ax_h.at[rows], ax.at[rows])]
            elif d[0] == "xc":
                blk = (pl.ds(0, 256), pl.ds(d[1] * 128, (d[2] - d[1]) * 128))
                pairs = [(ax_h.at[blk], ax.at[blk])]
            elif d[0] == "d":
                pairs = [(wd_hbm.bitcast(I32), wd)]
            elif d[0] == "v":
                pairs = [(wr_hbm, wr_ref), (gw_hbm, gw_ref)]
            elif d[0] == "wo":
                pairs = [(wo_hbm.bitcast(I32).at[:, pl.ds(j * 128, 128)], wo_raw.at[j]) for j in range(NT)]
            else:
                pairs = [(h.bitcast(I32), v) for h, v in ((wg_hbm, wg), (wu_hbm, wu))]
            cps[d] = [pltpu.make_async_copy(a, b, si.at[nsem + k]) for k, (a, b) in enumerate(pairs)]
            nsem += len(pairs)
            for c in cps[d]:
                c.start()

        lane = lax.broadcasted_iota(I32, (8, 128), 1)

        def permute_chunk(s, k0, k1):
            for jp in range(NT):
                src = (20 * (lane & 31) + 4 * jp + (lane >> 5)) & 127
                tile = (20 * ((13 * ((lane >> 2) - jp)) & 31) + 4 * jp + (lane & 3)) >> 7
                for r in range(k0 * 8, k1 * 8):
                    rows = pl.ds(r * 8, 8)
                    acc = wraw[s, rows, pl.ds(0, 128)]
                    for j in range(1, NT):
                        acc = jnp.where(tile == j, wraw[s, rows, pl.ds(j * 128, 128)], acc)
                    wp[rows, pl.ds(s * D + jp * 128, 128)] = jnp.take_along_axis(acc, src, axis=1)

        qscale = np.float32(DH ** -0.5 * np.log2(np.e))
        masked = np.float32(-1e9 * np.log2(np.e))

        def qkv_mm(s, r0, n):
            x = pltpu.bitcast(ax[pl.ds(r0 // 2, n // 2), :], BF16)
            y = jnp.dot(x, pltpu.bitcast(wp[:, s * D:(s + 1) * D], BF16), preferred_element_type=F32)
            if s == 0:
                y = y * qscale

            def store():
                p0 = r0 % ring
                for j in range(NT):
                    qkv[s * NT + j, pl.ds(p0 + HALO, n), :] = y[:, j * 128:(j + 1) * 128]
                    if s > 0 and p0 + n == ring and r0 + n < S:
                        qkv[s * NT + j, pl.ds(0, HALO), :] = y[n - HALO:, j * 128:(j + 1) * 128]
            return store

        att_done = 0

        def attn_steps():
            d1, d2, d3, d4 = dl
            N = (S // RG) * W
            nonlocal att_done
            a1, r1, a2, r2, ls, es, acc = {}, {}, {}, {}, {}, {}, {}
            for t in range(N + d1 + d2 + W + d3):
                yield min(S, (t // W + 1) * RG)
                if t < N:
                    g, w = divmod(t, W)
                    r = HALO + (g * RG) % ring
                    if w == 0:
                        q = [qkv[j, pl.ds(r, RG), :] for j in range(NT)]
                    pr = [q[j] * qkv[NT + j, pl.ds(r - DIL * w, RG), :] for j in range(NT)]
                    a1[t] = tree(add, pr) if qktree else (((pr[0] + pr[1]) + pr[2]) + pr[3]) + pr[4]
                    r1[t] = pltpu.roll(a1[t], 64, 1)
                u = t - d1
                if 0 <= u < N:
                    a2[u] = a1.pop(u) + r1.pop(u)
                    r2[u] = pltpu.roll(a2[u], 32, 1)
                u = t - d1 - d2
                if 0 <= u < N:
                    g, w = divmod(u, W)
                    a = a2.pop(u) + r2.pop(u)
                    if g * RG < DIL * w:
                        pos = lax.broadcasted_iota(I32, (RG, 128), 0) + g * RG
                        a = jnp.where(pos >= DIL * w, a, masked)
                    ls[u] = a
                    if w == W - 1:
                        l8 = [ls.pop(g * W + k) for k in range(W)]
                        m = tree(jnp.maximum, l8)
                        for k in range(W):
                            es[g * W + k] = jnp.exp2(l8[k] - m)
                u = t - d1 - d2 - (W - 1) - d3
                if 0 <= u < N:
                    g, w = divmod(u, W)
                    r = HALO + (g * RG) % ring
                    if w == 0:
                        den = tree(add, [es[g * W + k] for k in range(W)])
                        inv = pl.reciprocal(den, approx=True)
                    if w == d4 and newton:
                        inv = inv * (2.0 - den * inv)
                    e = es.pop(u)
                    for j in range(NT):
                        p = e * qkv[2 * NT + j, pl.ds(r - DIL * w, RG), :]
                        acc[j] = p if w == 0 else acc[j] + p
                    if w == W - 1:
                        o = [acc[j] * inv for j in range(NT)]
                        if RG >= 16:
                            for j in range(NT):
                                o_s[pl.ds(g * (RG // 2), RG // 2), pl.ds(j * 128, 128)] = pltpu.bitcast(o[j].astype(BF16), I32)
                        elif g % 2 == 0:
                            held = o
                        else:
                            for j in range(NT):
                                o2 = jnp.concatenate([held[j], o[j]], axis=0)
                                o_s[pl.ds((g - 1) * 4, 8), pl.ds(j * 128, 128)] = pltpu.bitcast(o2.astype(BF16), I32)
                            att_done = (g + 1) * RG

        racc = [jnp.zeros((8, 128), F32)] * 2
        gacc = list(racc)
        vecs = []

        def router(g):
            if not vecs:
                vecs.extend(jnp.broadcast_to(v[...].astype(F32).reshape(1, D), (8, D)) for v in (wr_ref, gw_ref))
            xf = pltpu.bitcast(ax[pl.ds(g * 8, 8), :], BF16).astype(F32)
            for p in range(2):
                n = 2 * g + p
                xp = xf[8 * p:8 * p + 8]
                rr = jnp.sum(xp * vecs[0], axis=1, keepdims=True)
                racc[n // 128] = jnp.where(lane == n % 128, rr, racc[n // 128])
                gl = jnp.sum(xp * vecs[1], axis=1, keepdims=True)
                gacc[n // 128] = jnp.where(lane == n % 128, gl, gacc[n // 128])

        def wo_gather(j, d2):
            ev = wo_raw[j, pl.ds(d2, H // 2, stride=DH), :]
            od = wo_raw[j, pl.ds(DH // 2 + d2, H // 2, stride=DH), :]
            cols = pl.ds(j * 128, 128)
            wop[pl.ds(d2 * 32, 16), cols] = (ev & 0xFFFF) | (od << 16)
            wop[pl.ds(d2 * 32 + 16, 16), cols] = lax.shift_right_logical(ev, 16) | (od & HI)

        sub = lax.broadcasted_iota(I32, (8, 128), 0)
        sel = {}

        def select():
            for p in range(2):
                g_s[p] = jax.nn.sigmoid(gacc[p])
            keys = []
            for p in range(2):
                rr = racc[p].astype(BF16).astype(F32)
                rr = jnp.where(rr == 0, np.float32(0), rr)
                bits = pltpu.bitcast(rr, I32)
                key = jnp.where(bits < 0, bits ^ np.int32(0x7FFF0000), bits)
                key = jnp.where(rr != rr, np.int32(-2**31), key)
                keys.append(key | (S - 1 - (1024 * p + 8 * lane + sub)))
            k1 = jnp.max(jnp.maximum(*keys))
            k2 = jnp.max(jnp.maximum(*[jnp.where(k == k1, np.int32(-2**31), k) for k in keys]))
            sel["idx"] = [S - 1 - (k & (S - 1)) for k in (k1, k2)]
            sel["keys"] = (k1, k2)
            subD = lax.broadcasted_iota(I32, (16, D), 0)
            for c, t in enumerate(sel["idx"]):
                blk = pltpu.bitcast(ax[pl.ds(pl.multiple_of((t >> 4) << 3, 8), 8), :], BF16).astype(F32)
                row = jnp.sum(jnp.where(subD == (t & 15), blk, 0.0), axis=0, keepdims=True)
                xsel[c] = jnp.broadcast_to(row, (8, D))

        pre = {}

        def gate_up(l):
            T = l // 8
            for m, w_ref in enumerate((wg, wu)):
                ww = w_ref[pl.ds(l * 8, 8), :]
                for p, wf in enumerate((ww << 16, ww & HI)):
                    wf = pltpu.bitcast(wf, F32)
                    here = lane - 2 * sub == 16 * (l % 8) + p
                    for c in range(2):
                        val = jnp.sum(wf * xsel[c], axis=1, keepdims=True)
                        pre[m, c] = jnp.where(here, val, pre.get((m, c), np.float32(0)))
            if l % 8 == 7 or l == F // 16 - 1:
                hh = jnp.concatenate([jax.nn.silu(pre.pop((0, c))) * pre.pop((1, c)) for c in range(2)], axis=0)
                hbuf[:, pl.ds(T * 128, 128)] = pltpu.bitcast(hh.astype(BF16), I32)

        def down():
            yy = jnp.dot(pltpu.bitcast(hbuf[:, pl.ds(0, F)], BF16), pltpu.bitcast(wd[...], BF16), preferred_element_type=F32)
            ys = []
            for c, k in enumerate(sel["keys"]):
                kb = jnp.full((1, 128), k & HI, I32)
                rs = jax.nn.sigmoid(pltpu.bitcast(jnp.where(kb < 0, kb ^ np.int32(0x7FFF0000), kb), F32))
                ys.append(jnp.sum(yy[8 * c:8 * c + 8], axis=0, keepdims=True) * jnp.concatenate([rs] * NT, axis=1))
            return sel["idx"], ys

        def patch(idx, yy):
            subD = lax.broadcasted_iota(I32, (16, D), 0)
            for c, t in enumerate(idx):
                rows = pl.ds(pl.multiple_of((t >> 4) << 3, 8), 8)
                blk = pltpu.bitcast(ax[rows, :], BF16).astype(F32)
                blk = jnp.where(subD == (t & 15), blk + yy[c], blk)
                ax[rows, :] = pltpu.bitcast(blk.astype(BF16), I32)

        cp_o = [pltpu.make_async_copy(out_s.at[pl.ds(r0 // 2, n // 2)], out_h.at[pl.ds(r0 // 2, n // 2)], so.at[i])
                for i, (r0, n) in enumerate(outs)]

        def out_block(r0, n):
            assert att_done >= r0 + n
            rows = pl.ds(r0 // 2, n // 2)
            a = jnp.dot(pltpu.bitcast(o_s[rows, :], BF16), pltpu.bitcast(wop[...], BF16), preferred_element_type=F32)
            b = pltpu.bitcast(ax[rows, :], BF16).astype(F32)
            g = g_rep[pl.ds(r0, n), :]
            g = jnp.concatenate([g] * NT, axis=1)
            out_s[rows, :] = pltpu.bitcast((b + g * (a - b)).astype(BF16), I32)

        for j in range(NT):
            qkv[NT + j, pl.ds(0, HALO), :] = jnp.zeros((HALO, 128), F32)
        att = attn_steps()
        need = next(att)
        pending = []

        def run_aux(r):
            if "rt" in r:
                for g in range(r["rt"][0] // 16, r["rt"][1] // 16):
                    router(g)
            if r.get("select"):
                select()
            for l in r.get("xp", ()):
                gate_up(l)
            if "gx" in r:
                gc = [g_s[0], g_s[1]]
                for m in range(r["gx"][0] // 8, r["gx"][1] // 8):
                    g_rep[pl.ds(m * 8, 8), :] = jnp.broadcast_to(gc[m // 128][:, m % 128:m % 128 + 1], (8, 128))
            for j in r.get("wo", ()):
                for d in range(DH // 2):
                    wo_gather(j, d)

        for k, r in enumerate(regions):
            with scope(str(k)):
                for d in r.get("wait", []):
                    for c in cps[d]:
                        c.wait()
                if r.get("name") not in merge:
                    pl.semaphore_signal(sbar, 1)
                    pl.semaphore_wait(sbar, 1)
                if r.get("patch"):
                    patch(*res)
                for p in r.get("perm", []):
                    permute_chunk(*p)
                for fn in pending:
                    fn()
                pending = []
                if "kmm" in r:
                    k0, k1 = r["kmm"]
                    y = jnp.dot(pltpu.bitcast(ax[pl.ds(0, 256), k0 * 128:k1 * 128], BF16),
                                pltpu.bitcast(wp[k0 * 64:k1 * 64, D:2 * D], BF16), preferred_element_type=F32)
                    for j in range(NT):
                        dst = (NT + j, pl.ds(HALO, 512), slice(None))
                        qkv[dst] = y[:, j * 128:(j + 1) * 128] + (qkv[dst] if k0 else 0.0)
                if auxpos == "start":
                    run_aux(r)
                mms = list(r.get("mm", []))
                if defer and mms and k + 1 < len(regions) and not r.get("halo"):
                    s_, r0, n = mms.pop()
                    if n > defer:
                        mms.append((s_, r0, n - defer))
                    for m in mms:
                        qkv_mm(*m)()
                    pending.append(qkv_mm(s_, r0 + n - min(n, defer), min(n, defer)))
                else:
                    for m in mms:
                        qkv_mm(*m)()
                if r.get("halo"):
                    for j in range(NT):
                        qkv[2 * NT + j, pl.ds(0, HALO), :] = jnp.broadcast_to(qkv[2 * NT + j, pl.ds(HALO, 1), :], (HALO, 128))
                late = [o for o in r.get("out", []) if att_done < sum(o)]
                for o in r.get("out", []):
                    if o not in late:
                        out_block(*o)
                if auxpos == "mid":
                    run_aux(r)
                while need is not None and need <= r.get("att", 0):
                    need = next(att, None)
                for o in late:
                    out_block(*o)
                if auxpos == "end":
                    run_aux(r)
                if r.get("ffn"):
                    res = down()
                for o in r.get("out", []):
                    cp_o[outs.index(o)].start()
        with scope("tail"):
            for c in cp_o:
                c.wait()

    def f(A_x, A_wqkv, A_wo, B_x, B_w_r, B_w_gate, B_w_up, B_w_down, gate_w):
        hbm = pl.BlockSpec(memory_space=pltpu.HBM)
        vm = pl.BlockSpec(memory_space=pltpu.VMEM)
        out = pl.pallas_call(
            kern,
            out_shape=jax.ShapeDtypeStruct((S, D), BF16),
            in_specs=[hbm] * 8,
            out_specs=hbm,
            scratch_shapes=[
                pltpu.VMEM((S // 2, D), I32),
                pltpu.VMEM((3, D // 2, D), I32), pltpu.VMEM((D // 2, 3 * D), I32),
                pltpu.VMEM((NT, D // 2, 128), I32), pltpu.VMEM((D // 2, D), I32),
                pltpu.VMEM((F // 2, D), I32), pltpu.VMEM((F // 2, D), I32), pltpu.VMEM((F // 2, D), I32),
                pltpu.VMEM((2, 8, D), F32), pltpu.VMEM((8, 1792), I32),
                pltpu.VMEM((3 * NT, HALO + ring, 128), F32),
                pltpu.VMEM((S // 2, D), I32), pltpu.VMEM((S // 2, D), I32),
                pltpu.VMEM((2, 8, 128), F32), pltpu.VMEM((S, 128), F32), pltpu.VMEM((D,), BF16), pltpu.VMEM((D,), BF16),
                pltpu.SemaphoreType.DMA((len(dma) + 7,)), pltpu.SemaphoreType.DMA((len(outs),)), pltpu.SemaphoreType.REGULAR,
            ],
            compiler_params=pltpu.CompilerParams(vmem_limit_bytes=100 * 2**20, flags=flags),
        )(A_x.reshape(S, D), A_wqkv, A_wo, B_w_r, B_w_gate.T, B_w_up.T, B_w_down, gate_w)
        return out.reshape(1, S, D)
    return f


_impl = make(**dict(merge=(2,6),xp={4:(0,54),5:(54,108)}))


@jax.jit
def pallas_gated_mix__sliding_local_dilated__moe_arch_mod__prompt_kernel(
    A_x, A_wqkv, A_wo, B_x, B_w_r, B_w_gate, B_w_up, B_w_down, gate_w
):
    return _impl(A_x, A_wqkv, A_wo, B_x, B_w_r, B_w_gate, B_w_up, B_w_down, gate_w)
```

```python
import contextlib
import numpy as np
import jax
import jax.numpy as jnp
from jax import lax
from jax.experimental import pallas as pl
from jax.experimental.pallas import tpu as pltpu

S, D, H, DH, W, DIL, F = 2048, 640, 32, 20, 8, 2, 1728
NT = D // 128
HALO = 16
PITCH = 20
F32, BF16, I32 = jnp.float32, jnp.bfloat16, jnp.int32
HI = np.int32(-65536)


def tree(f, xs):
    while len(xs) > 1:
        xs = [f(xs[k], xs[k + 1]) if k + 1 < len(xs) else xs[k] for k in range(0, len(xs), 2)]
    return xs[0]


def add(a, b):
    return a + b


def plan(att=(0, 240, 480, 720, 976, 1232, 1520, 1792, 2048), x2=896, rt=(1536, 2048), wo=3, sel_at=3,
         xp={4: (0, 54), 5: (54, 108)}, ffn=6, kc=2, dw=5, mmr=128, so=(1, 0, 2), r0=(256, 512), wk=(3, 5),
         ob=((256, 256, 256), (256, 256, 256), (256, 128), (128,))):
    if kc:
        dma = [("xc", 0, kc), ("w", 1, 0, kc), ("xc", kc, 5), ("w", 1, kc, 5), ("v",)]
        R = [dict(wait=dma[:2], perm=[(1, 0, kc)], kmm=(0, kc)), dict(wait=dma[2:], perm=[(1, kc, 5)], kmm=(kc, 5), rt=(0, r0[0]))]
        R.append(dict(wait=[("w", 0, 0, 5)], perm=[(0, 0, 5)], mm=[(0, 0, 256)], rt=r0))
    else:
        dma = [("w", 1, a, b) for a, b in zip((0,) + wk[:-1], wk)] + [("x", 0, 256), ("x", 256, 512)]
        R = [dict(wait=[d], perm=[d[1:]]) for d in dma[:len(wk)]]
        R.append(dict(wait=[("x", 0, 256)], mm=[(1, 0, 256)]))
        R.append(dict(wait=[("x", 256, 512)], mm=[(1, 256, 128)]))
        R.append(dict(wait=[("w", 0, 0, 5)], perm=[(0, 0, 5)], mm=[(1, 384, 128), (0, 0, 256)]))
    dma += [("w", 0, 0, 5), ("w", 2, 0, 5), ("x", 512, x2), ("x", x2, S), ("wo",), ("f",), ("d",)]
    R.append(dict(wait=[("w", 2, 0, 5), ("x", 512, x2)], perm=[(2, 0, 5)], halo=True, rt=(r0[1], x2), att=att[0],
                  mm=[(2, 0, 256), (0, 256, 256), (2, 256, 256)], name=0))
    nr = x2
    for i in range(1, 7):
        r = dict(mm=[(s, 256 + 256 * i + a, mmr) for s in so for a in range(0, 256, mmr)], att=att[i], wait=[], name=i)
        if i == 1:
            r["wait"] += [("x", x2, S), ("wo",)]
        if i <= len(rt):
            r["rt"] = (nr, rt[i - 1]); nr = rt[i - 1]
        if i == wo:
            r["wo"] = range(NT)
        if i == sel_at:
            r["select"] = True
        if i in xp:
            r["xp"] = range(*xp[i])
        if i == min(xp):
            r["wait"].append(("f",))
        if i == dw:
            r["wait"].append(("d",))
        if i == ffn:
            r["ffn"] = True
        R.append(r)
    r0 = 0
    for k, blocks in enumerate(ob):
        r = dict(out=[], patch=k == 0, name=7 + k)
        for n in blocks:
            r["out"].append((r0, n)); r0 += n
        if 7 + k < len(att):
            r["att"] = att[7 + k]
        R.append(r)
    for a, b in zip(R[:-1], R[1:]):
        if "out" in b:
            a["gx"] = (b["out"][0][0], sum(b["out"][-1]))
    assert r0 == S and nr == S
    return dma, R


def make(RG=8, flags=None, scopes=False, dl=(6, 6, 6, 4), qktree=False, newton=True, merge=(2, 6), defer=0, ring=S, auxpos="start", **kw):
    dma, regions = plan(**kw)
    outs = [o for r in regions for o in r.get("out", [])]
    scope = (lambda n: jax.named_scope("Z" + n)) if scopes else (lambda n: contextlib.nullcontext())

    def kern(ax_hbm, wqkv_hbm, wo_hbm, wr_hbm, wg_hbm, wu_hbm, wd_hbm, gw_hbm, out_hbm,
             ax, wraw, wp, wo_raw, wop, wg, wu, wd, xsel, hbuf, qkv, o_s, out_s, g_s, g_rep, wr_ref, gw_ref, si, so, sbar):
        ax_h, wqkv_h, out_h = (r.bitcast(I32) for r in (ax_hbm, wqkv_hbm, out_hbm))
        cps, nsem = {}, 0
        for d in dma:
            if d[0] == "w":
                rows = pl.ds(d[2] * 64, (d[3] - d[2]) * 64)
                pairs = [(wqkv_h.at[rows, pl.ds(d[1] * D, D)], wraw.at[d[1], rows])]
            elif d[0] == "x":
                rows = pl.ds(d[1] // 2, (d[2] - d[1]) // 2)
                pairs = [(ax_h.at[rows], ax.at[rows])]
            elif d[0] == "xc":
                blk = (pl.ds(0, 256), pl.ds(d[1] * 128, (d[2] - d[1]) * 128))
                pairs = [(ax_h.at[blk], ax.at[blk])]
            elif d[0] == "d":
                pairs = [(wd_hbm.bitcast(I32), wd)]
            elif d[0] == "v":
                pairs = [(wr_hbm, wr_ref), (gw_hbm, gw_ref)]
            elif d[0] == "wo":
                pairs = [(wo_hbm.bitcast(I32).at[:, pl.ds(j * 128, 128)], wo_raw.at[j]) for j in range(NT)]
            else:
                pairs = [(h.bitcast(I32), v) for h, v in ((wg_hbm, wg), (wu_hbm, wu))]
            cps[d] = [pltpu.make_async_copy(a, b, si.at[nsem + k]) for k, (a, b) in enumerate(pairs)]
            nsem += len(pairs)
            for c in cps[d]:
                c.start()

        lane = lax.broadcasted_iota(I32, (8, 128), 1)

        def permute_chunk(s, k0, k1):
            for jp in range(NT):
                src = (20 * (lane & 31) + 4 * jp + (lane >> 5)) & 127
                tile = (20 * ((13 * ((lane >> 2) - jp)) & 31) + 4 * jp + (lane & 3)) >> 7
                for r in range(k0 * 8, k1 * 8):
                    rows = pl.ds(r * 8, 8)
                    acc = wraw[s, rows, pl.ds(0, 128)]
                    for j in range(1, NT):
                        acc = jnp.where(tile == j, wraw[s, rows, pl.ds(j * 128, 128)], acc)
                    wp[rows, pl.ds(s * D + jp * 128, 128)] = jnp.take_along_axis(acc, src, axis=1)

        qscale = np.float32(DH ** -0.5 * np.log2(np.e))
        masked = np.float32(-1e9 * np.log2(np.e))

        def qkv_mm(s, r0, n):
            x = pltpu.bitcast(ax[pl.ds(r0 // 2, n // 2), :], BF16)
            if s == 3:
                y3 = jnp.dot(x, pltpu.bitcast(wp[...], BF16), preferred_element_type=F32)
                for c in range(3 * NT):
                    yc = y3[:, c * 128:(c + 1) * 128]
                    qkv[c, pl.ds(r0 + HALO, n), :] = yc * qscale if c < NT else yc
                return lambda: None
            y = jnp.dot(x, pltpu.bitcast(wp[:, s * D:(s + 1) * D], BF16), preferred_element_type=F32)
            if s == 0:
                y = y * qscale

            def store():
                p0 = r0 % ring
                for j in range(NT):
                    qkv[s * NT + j, pl.ds(p0 + HALO, n), :] = y[:, j * 128:(j + 1) * 128]
                    if s > 0 and p0 + n == ring and r0 + n < S:
                        qkv[s * NT + j, pl.ds(0, HALO), :] = y[n - HALO:, j * 128:(j + 1) * 128]
            return store

        att_done = 0

        def attn_steps():
            d1, d2, d3, d4 = dl
            N = (S // RG) * W
            nonlocal att_done
            a1, r1, a2, r2, ls, es, acc = {}, {}, {}, {}, {}, {}, {}
            for t in range(N + d1 + d2 + W + d3):
                yield min(S, (t // W + 1) * RG)
                if t < N:
                    g, w = divmod(t, W)
                    r = HALO + (g * RG) % ring
                    if w == 0:
                        q = [qkv[j, pl.ds(r, RG), :] for j in range(NT)]
                    pr = [q[j] * qkv[NT + j, pl.ds(r - DIL * w, RG), :] for j in range(NT)]
                    a1[t] = tree(add, pr) if qktree else (((pr[0] + pr[1]) + pr[2]) + pr[3]) + pr[4]
                    r1[t] = pltpu.roll(a1[t], 64, 1)
                u = t - d1
                if 0 <= u < N:
                    a2[u] = a1.pop(u) + r1.pop(u)
                    r2[u] = pltpu.roll(a2[u], 32, 1)
                u = t - d1 - d2
                if 0 <= u < N:
                    g, w = divmod(u, W)
                    a = a2.pop(u) + r2.pop(u)
                    if g * RG < DIL * w:
                        pos = lax.broadcasted_iota(I32, (RG, 128), 0) + g * RG
                        a = jnp.where(pos >= DIL * w, a, masked)
                    ls[u] = a
                    if w == W - 1:
                        l8 = [ls.pop(g * W + k) for k in range(W)]
                        m = tree(jnp.maximum, l8)
                        for k in range(W):
                            es[g * W + k] = jnp.exp2(l8[k] - m)
                u = t - d1 - d2 - (W - 1) - d3
                if 0 <= u < N:
                    g, w = divmod(u, W)
                    r = HALO + (g * RG) % ring
                    if w == 0:
                        den = tree(add, [es[g * W + k] for k in range(W)])
                        inv = pl.reciprocal(den, approx=True)
                    if w == d4 and newton:
                        inv = inv * (2.0 - den * inv)
                    e = es.pop(u)
                    for j in range(NT):
                        p = e * qkv[2 * NT + j, pl.ds(r - DIL * w, RG), :]
                        acc[j] = p if w == 0 else acc[j] + p
                    if w == W - 1:
                        o = [acc[j] * inv for j in range(NT)]
                        if RG >= 16:
                            for j in range(NT):
                                o_s[pl.ds(g * (RG // 2), RG // 2), pl.ds(j * 128, 128)] = pltpu.bitcast(o[j].astype(BF16), I32)
                        elif g % 2 == 0:
                            held = o
                        else:
                            for j in range(NT):
                                o2 = jnp.concatenate([held[j], o[j]], axis=0)
                                o_s[pl.ds((g - 1) * 4, 8), pl.ds(j * 128, 128)] = pltpu.bitcast(o2.astype(BF16), I32)
                            att_done = (g + 1) * RG

        racc = [jnp.zeros((8, 128), F32)] * 2
        gacc = list(racc)
        vecs = []

        def router(g):
            if not vecs:
                vecs.extend(jnp.broadcast_to(v[...].astype(F32).reshape(1, D), (8, D)) for v in (wr_ref, gw_ref))
            xf = pltpu.bitcast(ax[pl.ds(g * 8, 8), :], BF16).astype(F32)
            for p in range(2):
                n = 2 * g + p
                xp = xf[8 * p:8 * p + 8]
                rr = jnp.sum(xp * vecs[0], axis=1, keepdims=True)
                racc[n // 128] = jnp.where(lane == n % 128, rr, racc[n // 128])
                gl = jnp.sum(xp * vecs[1], axis=1, keepdims=True)
                gacc[n // 128] = jnp.where(lane == n % 128, gl, gacc[n // 128])

        def wo_gather(j, d2):
            ev = wo_raw[j, pl.ds(d2, H // 2, stride=DH), :]
            od = wo_raw[j, pl.ds(DH // 2 + d2, H // 2, stride=DH), :]
            cols = pl.ds(j * 128, 128)
            wop[pl.ds(d2 * 32, 16), cols] = (ev & 0xFFFF) | (od << 16)
            wop[pl.ds(d2 * 32 + 16, 16), cols] = lax.shift_right_logical(ev, 16) | (od & HI)

        sub = lax.broadcasted_iota(I32, (8, 128), 0)
        sel = {}

        def select():
            for p in range(2):
                g_s[p] = jax.nn.sigmoid(gacc[p])
            keys = []
            for p in range(2):
                rr = racc[p].astype(BF16).astype(F32)
                rr = jnp.where(rr == 0, np.float32(0), rr)
                bits = pltpu.bitcast(rr, I32)
                key = jnp.where(bits < 0, bits ^ np.int32(0x7FFF0000), bits)
                key = jnp.where(rr != rr, np.int32(-2**31), key)
                keys.append(key | (S - 1 - (1024 * p + 8 * lane + sub)))
            k1 = jnp.max(jnp.maximum(*keys))
            k2 = jnp.max(jnp.maximum(*[jnp.where(k == k1, np.int32(-2**31), k) for k in keys]))
            sel["idx"] = [S - 1 - (k & (S - 1)) for k in (k1, k2)]
            sel["keys"] = (k1, k2)
            subD = lax.broadcasted_iota(I32, (16, D), 0)
            for c, t in enumerate(sel["idx"]):
                blk = pltpu.bitcast(ax[pl.ds(pl.multiple_of((t >> 4) << 3, 8), 8), :], BF16).astype(F32)
                row = jnp.sum(jnp.where(subD == (t & 15), blk, 0.0), axis=0, keepdims=True)
                xsel[c] = jnp.broadcast_to(row, (8, D))

        pre = {}

        def gate_up(l):
            T = l // 8
            for m, w_ref in enumerate((wg, wu)):
                ww = w_ref[pl.ds(l * 8, 8), :]
                for p, wf in enumerate((ww << 16, ww & HI)):
                    wf = pltpu.bitcast(wf, F32)
                    here = lane - 2 * sub == 16 * (l % 8) + p
                    for c in range(2):
                        val = jnp.sum(wf * xsel[c], axis=1, keepdims=True)
                        pre[m, c] = jnp.where(here, val, pre.get((m, c), np.float32(0)))
            if l % 8 == 7 or l == F // 16 - 1:
                hh = jnp.concatenate([jax.nn.silu(pre.pop((0, c))) * pre.pop((1, c)) for c in range(2)], axis=0)
                hbuf[:, pl.ds(T * 128, 128)] = pltpu.bitcast(hh.astype(BF16), I32)

        def down():
            yy = jnp.dot(pltpu.bitcast(hbuf[:, pl.ds(0, F)], BF16), pltpu.bitcast(wd[...], BF16), preferred_element_type=F32)
            ys = []
            for c, k in enumerate(sel["keys"]):
                kb = jnp.full((1, 128), k & HI, I32)
                rs = jax.nn.sigmoid(pltpu.bitcast(jnp.where(kb < 0, kb ^ np.int32(0x7FFF0000), kb), F32))
                ys.append(jnp.sum(yy[8 * c:8 * c + 8], axis=0, keepdims=True) * jnp.concatenate([rs] * NT, axis=1))
            return sel["idx"], ys

        def patch(idx, yy):
            subD = lax.broadcasted_iota(I32, (16, D), 0)
            for c, t in enumerate(idx):
                rows = pl.ds(pl.multiple_of((t >> 4) << 3, 8), 8)
                blk = pltpu.bitcast(ax[rows, :], BF16).astype(F32)
                blk = jnp.where(subD == (t & 15), blk + yy[c], blk)
                ax[rows, :] = pltpu.bitcast(blk.astype(BF16), I32)

        cp_o = [pltpu.make_async_copy(out_s.at[pl.ds(r0 // 2, n // 2)], out_h.at[pl.ds(r0 // 2, n // 2)], so.at[i])
                for i, (r0, n) in enumerate(outs)]

        def out_block(r0, n):
            assert att_done >= r0 + n
            rows = pl.ds(r0 // 2, n // 2)
            a = jnp.dot(pltpu.bitcast(o_s[rows, :], BF16), pltpu.bitcast(wop[...], BF16), preferred_element_type=F32)
            b = pltpu.bitcast(ax[rows, :], BF16).astype(F32)
            g = g_rep[pl.ds(r0, n), :]
            g = jnp.concatenate([g] * NT, axis=1)
            out_s[rows, :] = pltpu.bitcast((b + g * (a - b)).astype(BF16), I32)

        for j in range(NT):
            qkv[NT + j, pl.ds(0, HALO), :] = jnp.zeros((HALO, 128), F32)
        att = attn_steps()
        need = next(att)
        pending = []

        def run_aux(r):
            if "rt" in r:
                for g in range(r["rt"][0] // 16, r["rt"][1] // 16):
                    router(g)
            if r.get("select"):
                select()
            for l in () if r.get("select") else r.get("xp", ()):
                gate_up(l)
            if "gx" in r:
                gc = [g_s[0], g_s[1]]
                for m in range(r["gx"][0] // 8, r["gx"][1] // 8):
                    g_rep[pl.ds(m * 8, 8), :] = jnp.broadcast_to(gc[m // 128][:, m % 128:m % 128 + 1], (8, 128))
            for j in r.get("wo", ()):
                for d in range(DH // 2):
                    wo_gather(j, d)

        for k, r in enumerate(regions):
            with scope(str(k)):
                for d in r.get("wait", []):
                    for c in cps[d]:
                        c.wait()
                if r.get("name") not in merge:
                    pl.semaphore_signal(sbar, 1)
                    pl.semaphore_wait(sbar, 1)
                if r.get("patch"):
                    patch(*res)
                for p in r.get("perm", []):
                    permute_chunk(*p)
                for fn in pending:
                    fn()
                pending = []
                if "kmm" in r:
                    k0, k1 = r["kmm"]
                    y = jnp.dot(pltpu.bitcast(ax[pl.ds(0, 256), k0 * 128:k1 * 128], BF16),
                                pltpu.bitcast(wp[k0 * 64:k1 * 64, D:2 * D], BF16), preferred_element_type=F32)
                    for j in range(NT):
                        dst = (NT + j, pl.ds(HALO, 512), slice(None))
                        qkv[dst] = y[:, j * 128:(j + 1) * 128] + (qkv[dst] if k0 else 0.0)
                if auxpos == "start":
                    run_aux(r)
                mms = list(r.get("mm", []))
                if defer and mms and k + 1 < len(regions) and not r.get("halo"):
                    s_, r0, n = mms.pop()
                    if n > defer:
                        mms.append((s_, r0, n - defer))
                    for m in mms:
                        qkv_mm(*m)()
                    pending.append(qkv_mm(s_, r0 + n - min(n, defer), min(n, defer)))
                else:
                    for m in mms:
                        qkv_mm(*m)()
                if r.get("halo"):
                    for j in range(NT):
                        qkv[2 * NT + j, pl.ds(0, HALO), :] = jnp.broadcast_to(qkv[2 * NT + j, pl.ds(HALO, 1), :], (HALO, 128))
                late = [o for o in r.get("out", []) if att_done < sum(o)]
                for o in r.get("out", []):
                    if o not in late:
                        out_block(*o)
                if auxpos == "mid":
                    run_aux(r)
                while need is not None and need <= r.get("att", 0):
                    need = next(att, None)
                for l in r.get("xp", ()) if r.get("select") else ():
                    gate_up(l)
                for o in late:
                    out_block(*o)
                if auxpos == "end":
                    run_aux(r)
                if r.get("ffn"):
                    res = down()
                for o in r.get("out", []):
                    cp_o[outs.index(o)].start()
        with scope("tail"):
            for c in cp_o:
                c.wait()

    def f(A_x, A_wqkv, A_wo, B_x, B_w_r, B_w_gate, B_w_up, B_w_down, gate_w):
        hbm = pl.BlockSpec(memory_space=pltpu.HBM)
        vm = pl.BlockSpec(memory_space=pltpu.VMEM)
        out = pl.pallas_call(
            kern,
            out_shape=jax.ShapeDtypeStruct((S, D), BF16),
            in_specs=[hbm] * 8,
            out_specs=hbm,
            scratch_shapes=[
                pltpu.VMEM((S // 2, D), I32),
                pltpu.VMEM((3, D // 2, D), I32), pltpu.VMEM((D // 2, 3 * D), I32),
                pltpu.VMEM((NT, D // 2, 128), I32), pltpu.VMEM((D // 2, D), I32),
                pltpu.VMEM((F // 2, D), I32), pltpu.VMEM((F // 2, D), I32), pltpu.VMEM((F // 2, D), I32),
                pltpu.VMEM((2, 8, D), F32), pltpu.VMEM((8, 1792), I32),
                pltpu.VMEM((3 * NT, HALO + ring, 128), F32),
                pltpu.VMEM((S // 2, D), I32), pltpu.VMEM((S // 2, D), I32),
                pltpu.VMEM((2, 8, 128), F32), pltpu.VMEM((S, 128), F32), pltpu.VMEM((D,), BF16), pltpu.VMEM((D,), BF16),
                pltpu.SemaphoreType.DMA((len(dma) + 7,)), pltpu.SemaphoreType.DMA((len(outs),)), pltpu.SemaphoreType.REGULAR,
            ],
            compiler_params=pltpu.CompilerParams(vmem_limit_bytes=100 * 2**20, flags=flags),
        )(A_x.reshape(S, D), A_wqkv, A_wo, B_w_r, B_w_gate.T, B_w_up.T, B_w_down, gate_w)
        return out.reshape(1, S, D)
    return f


_impl = make(**dict())


@jax.jit
def pallas_gated_mix__sliding_local_dilated__moe_arch_mod__prompt_kernel(
    A_x, A_wqkv, A_wo, B_x, B_w_r, B_w_gate, B_w_up, B_w_down, gate_w
):
    return _impl(A_x, A_wqkv, A_wo, B_x, B_w_r, B_w_gate, B_w_up, B_w_down, gate_w)
```

```python
import contextlib
import numpy as np
import jax
import jax.numpy as jnp
from jax import lax
from jax.experimental import pallas as pl
from jax.experimental.pallas import tpu as pltpu

S, D, H, DH, W, DIL, F = 2048, 640, 32, 20, 8, 2, 1728
NT = D // 128
HALO = 16
PITCH = 20
F32, BF16, I32 = jnp.float32, jnp.bfloat16, jnp.int32
HI = np.int32(-65536)


def tree(f, xs):
    while len(xs) > 1:
        xs = [f(xs[k], xs[k + 1]) if k + 1 < len(xs) else xs[k] for k in range(0, len(xs), 2)]
    return xs[0]


def add(a, b):
    return a + b


def plan(att=(0, 256, 512, 816, 1008, 1200, 1504, 1776, 2048), x2=896, rt=(1536, 2048), wo=3, sel_at=3,
         xp={4: (0, 54), 5: (54, 108)}, ffn=6, kc=2, dw=5, pmr=128, po=((0, 256), (2, 0), (2, 256)), ks=(512, 384), mmr=128, so=(1, 0, 2), r0=(256, 512), wk=(3, 5),
         ob=((256, 256, 256), (256, 256, 256), (256, 128), (128,))):
    if kc:
        dma = [("xc", 0, kc), ("w", 1, 0, kc), ("xc", kc, 5), ("w", 1, kc, 5), ("v",)]
        R = [dict(wait=dma[:2], perm=[(1, 0, kc)], kmm=[(0, kc, 0, ks[0])]), dict(wait=dma[2:], perm=[(1, kc, 5)], kmm=[(0, kc, ks[0], 512), (kc, 5, 0, ks[1])], rt=(0, r0[0]))]
        R.append(dict(wait=[("w", 0, 0, 5)], perm=[(0, 0, 5)], kmm=[(kc, 5, ks[1], 512)], mm=[(0, a, pmr) for a in range(0, 256, pmr)], rt=r0))
    else:
        dma = [("w", 1, a, b) for a, b in zip((0,) + wk[:-1], wk)] + [("x", 0, 256), ("x", 256, 512)]
        R = [dict(wait=[d], perm=[d[1:]]) for d in dma[:len(wk)]]
        R.append(dict(wait=[("x", 0, 256)], mm=[(1, 0, 256)]))
        R.append(dict(wait=[("x", 256, 512)], mm=[(1, 256, 128)]))
        R.append(dict(wait=[("w", 0, 0, 5)], perm=[(0, 0, 5)], mm=[(1, 384, 128), (0, 0, 256)]))
    dma += [("w", 0, 0, 5), ("w", 2, 0, 5), ("x", 512, x2), ("x", x2, S), ("wo",), ("f",), ("d",)]
    R.append(dict(wait=[("w", 2, 0, 5), ("x", 512, x2)], perm=[(2, 0, 5)], halo=True, rt=(r0[1], x2), att=att[0],
                  mm=[(s, b + a, pmr) for s, b in po for a in range(0, 256, pmr)], name=0))
    nr = x2
    for i in range(1, 7):
        r = dict(mm=[(s, 256 + 256 * i + a, mmr) for s in so for a in range(0, 256, mmr)], att=att[i], wait=[], name=i)
        if i == 1:
            r["wait"] += [("x", x2, S), ("wo",)]
        if i <= len(rt):
            r["rt"] = (nr, rt[i - 1]); nr = rt[i - 1]
        if i == wo:
            r["wo"] = range(NT)
        if i == sel_at:
            r["select"] = True
        if i in xp:
            r["xp"] = range(*xp[i])
        if i == min(xp):
            r["wait"].append(("f",))
        if i == dw:
            r["wait"].append(("d",))
        if i == ffn:
            r["ffn"] = True
        R.append(r)
    r0 = 0
    for k, blocks in enumerate(ob):
        r = dict(out=[], patch=k == 0, name=7 + k)
        for n in blocks:
            r["out"].append((r0, n)); r0 += n
        if 7 + k < len(att):
            r["att"] = att[7 + k]
        R.append(r)
    for a, b in zip(R[:-1], R[1:]):
        if "out" in b:
            a["gx"] = (b["out"][0][0], sum(b["out"][-1]))
    assert r0 == S and nr == S
    return dma, R


def make(RG=8, flags=None, scopes=False, dl=(6, 6, 6, 4), qktree=False, newton=True, merge=(2, 5, 6), defer=0, kmr=128, ring=S, auxpos="start", **kw):
    dma, regions = plan(**kw)
    outs = [o for r in regions for o in r.get("out", [])]
    scope = (lambda n: jax.named_scope("Z" + n)) if scopes else (lambda n: contextlib.nullcontext())

    def kern(ax_hbm, wqkv_hbm, wo_hbm, wr_hbm, wg_hbm, wu_hbm, wd_hbm, gw_hbm, out_hbm,
             ax, wraw, wp, wo_raw, wop, wg, wu, wd, xsel, hbuf, qkv, o_s, out_s, g_s, g_rep, wr_ref, gw_ref, si, so, sbar):
        ax_h, wqkv_h, out_h = (r.bitcast(I32) for r in (ax_hbm, wqkv_hbm, out_hbm))
        cps, nsem = {}, 0
        for d in dma:
            if d[0] == "w":
                rows = pl.ds(d[2] * 64, (d[3] - d[2]) * 64)
                pairs = [(wqkv_h.at[rows, pl.ds(d[1] * D, D)], wraw.at[d[1], rows])]
            elif d[0] == "x":
                rows = pl.ds(d[1] // 2, (d[2] - d[1]) // 2)
                pairs = [(ax_h.at[rows], ax.at[rows])]
            elif d[0] == "xc":
                blk = (pl.ds(0, 256), pl.ds(d[1] * 128, (d[2] - d[1]) * 128))
                pairs = [(ax_h.at[blk], ax.at[blk])]
            elif d[0] == "d":
                pairs = [(wd_hbm.bitcast(I32), wd)]
            elif d[0] == "v":
                pairs = [(wr_hbm, wr_ref), (gw_hbm, gw_ref)]
            elif d[0] == "wo":
                pairs = [(wo_hbm.bitcast(I32).at[:, pl.ds(j * 128, 128)], wo_raw.at[j]) for j in range(NT)]
            else:
                pairs = [(h.bitcast(I32), v) for h, v in ((wg_hbm, wg), (wu_hbm, wu))]
            cps[d] = [pltpu.make_async_copy(a, b, si.at[nsem + k]) for k, (a, b) in enumerate(pairs)]
            nsem += len(pairs)
            for c in cps[d]:
                c.start()

        lane = lax.broadcasted_iota(I32, (8, 128), 1)

        def permute_chunk(s, k0, k1):
            for jp in range(NT):
                src = (20 * (lane & 31) + 4 * jp + (lane >> 5)) & 127
                tile = (20 * ((13 * ((lane >> 2) - jp)) & 31) + 4 * jp + (lane & 3)) >> 7
                for r in range(k0 * 8, k1 * 8):
                    rows = pl.ds(r * 8, 8)
                    acc = wraw[s, rows, pl.ds(0, 128)]
                    for j in range(1, NT):
                        acc = jnp.where(tile == j, wraw[s, rows, pl.ds(j * 128, 128)], acc)
                    wp[rows, pl.ds(s * D + jp * 128, 128)] = jnp.take_along_axis(acc, src, axis=1)

        qscale = np.float32(DH ** -0.5 * np.log2(np.e))
        masked = np.float32(-1e9 * np.log2(np.e))

        def qkv_mm(s, r0, n):
            x = pltpu.bitcast(ax[pl.ds(r0 // 2, n // 2), :], BF16)
            if s == 3:
                y3 = jnp.dot(x, pltpu.bitcast(wp[...], BF16), preferred_element_type=F32)
                for c in range(3 * NT):
                    yc = y3[:, c * 128:(c + 1) * 128]
                    qkv[c, pl.ds(r0 + HALO, n), :] = yc * qscale if c < NT else yc
                return lambda: None
            y = jnp.dot(x, pltpu.bitcast(wp[:, s * D:(s + 1) * D], BF16), preferred_element_type=F32)
            if s == 0:
                y = y * qscale

            def store():
                p0 = r0 % ring
                for j in range(NT):
                    qkv[s * NT + j, pl.ds(p0 + HALO, n), :] = y[:, j * 128:(j + 1) * 128]
                    if s > 0 and p0 + n == ring and r0 + n < S:
                        qkv[s * NT + j, pl.ds(0, HALO), :] = y[n - HALO:, j * 128:(j + 1) * 128]
            return store

        att_done = 0

        def attn_steps():
            d1, d2, d3, d4 = dl
            N = (S // RG) * W
            nonlocal att_done
            a1, r1, a2, r2, ls, es, acc = {}, {}, {}, {}, {}, {}, {}
            for t in range(N + d1 + d2 + W + d3):
                yield min(S, (t // W + 1) * RG)
                if t < N:
                    g, w = divmod(t, W)
                    r = HALO + (g * RG) % ring
                    if w == 0:
                        q = [qkv[j, pl.ds(r, RG), :] for j in range(NT)]
                    pr = [q[j] * qkv[NT + j, pl.ds(r - DIL * w, RG), :] for j in range(NT)]
                    a1[t] = tree(add, pr) if qktree else (((pr[0] + pr[1]) + pr[2]) + pr[3]) + pr[4]
                    r1[t] = pltpu.roll(a1[t], 64, 1)
                u = t - d1
                if 0 <= u < N:
                    a2[u] = a1.pop(u) + r1.pop(u)
                    r2[u] = pltpu.roll(a2[u], 32, 1)
                u = t - d1 - d2
                if 0 <= u < N:
                    g, w = divmod(u, W)
                    a = a2.pop(u) + r2.pop(u)
                    if g * RG < DIL * w:
                        pos = lax.broadcasted_iota(I32, (RG, 128), 0) + g * RG
                        a = jnp.where(pos >= DIL * w, a, masked)
                    ls[u] = a
                    if w == W - 1:
                        l8 = [ls.pop(g * W + k) for k in range(W)]
                        m = tree(jnp.maximum, l8)
                        for k in range(W):
                            es[g * W + k] = jnp.exp2(l8[k] - m)
                u = t - d1 - d2 - (W - 1) - d3
                if 0 <= u < N:
                    g, w = divmod(u, W)
                    r = HALO + (g * RG) % ring
                    if w == 0:
                        den = tree(add, [es[g * W + k] for k in range(W)])
                        inv = pl.reciprocal(den, approx=True)
                    if w == d4 and newton:
                        inv = inv * (2.0 - den * inv)
                    e = es.pop(u)
                    for j in range(NT):
                        p = e * qkv[2 * NT + j, pl.ds(r - DIL * w, RG), :]
                        acc[j] = p if w == 0 else acc[j] + p
                    if w == W - 1:
                        o = [acc[j] * inv for j in range(NT)]
                        if RG >= 16:
                            for j in range(NT):
                                o_s[pl.ds(g * (RG // 2), RG // 2), pl.ds(j * 128, 128)] = pltpu.bitcast(o[j].astype(BF16), I32)
                        elif g % 2 == 0:
                            held = o
                        else:
                            for j in range(NT):
                                o2 = jnp.concatenate([held[j], o[j]], axis=0)
                                o_s[pl.ds((g - 1) * 4, 8), pl.ds(j * 128, 128)] = pltpu.bitcast(o2.astype(BF16), I32)
                            att_done = (g + 1) * RG

        racc = [jnp.zeros((8, 128), F32)] * 2
        gacc = list(racc)
        vecs = []

        def router(g):
            if not vecs:
                vecs.extend(jnp.broadcast_to(v[...].astype(F32).reshape(1, D), (8, D)) for v in (wr_ref, gw_ref))
            xf = pltpu.bitcast(ax[pl.ds(g * 8, 8), :], BF16).astype(F32)
            for p in range(2):
                n = 2 * g + p
                xp = xf[8 * p:8 * p + 8]
                rr = jnp.sum(xp * vecs[0], axis=1, keepdims=True)
                racc[n // 128] = jnp.where(lane == n % 128, rr, racc[n // 128])
                gl = jnp.sum(xp * vecs[1], axis=1, keepdims=True)
                gacc[n // 128] = jnp.where(lane == n % 128, gl, gacc[n // 128])

        def wo_gather(j, d2):
            ev = wo_raw[j, pl.ds(d2, H // 2, stride=DH), :]
            od = wo_raw[j, pl.ds(DH // 2 + d2, H // 2, stride=DH), :]
            cols = pl.ds(j * 128, 128)
            wop[pl.ds(d2 * 32, 16), cols] = (ev & 0xFFFF) | (od << 16)
            wop[pl.ds(d2 * 32 + 16, 16), cols] = lax.shift_right_logical(ev, 16) | (od & HI)

        sub = lax.broadcasted_iota(I32, (8, 128), 0)
        sel = {}

        def select():
            for p in range(2):
                g_s[p] = jax.nn.sigmoid(gacc[p])
            keys = []
            for p in range(2):
                rr = racc[p].astype(BF16).astype(F32)
                rr = jnp.where(rr == 0, np.float32(0), rr)
                bits = pltpu.bitcast(rr, I32)
                key = jnp.where(bits < 0, bits ^ np.int32(0x7FFF0000), bits)
                key = jnp.where(rr != rr, np.int32(-2**31), key)
                keys.append(key | (S - 1 - (1024 * p + 8 * lane + sub)))
            k1 = jnp.max(jnp.maximum(*keys))
            k2 = jnp.max(jnp.maximum(*[jnp.where(k == k1, np.int32(-2**31), k) for k in keys]))
            sel["idx"] = [S - 1 - (k & (S - 1)) for k in (k1, k2)]
            sel["keys"] = (k1, k2)
            subD = lax.broadcasted_iota(I32, (16, D), 0)
            for c, t in enumerate(sel["idx"]):
                blk = pltpu.bitcast(ax[pl.ds(pl.multiple_of((t >> 4) << 3, 8), 8), :], BF16).astype(F32)
                row = jnp.sum(jnp.where(subD == (t & 15), blk, 0.0), axis=0, keepdims=True)
                xsel[c] = jnp.broadcast_to(row, (8, D))

        pre = {}

        def gate_up(l):
            T = l // 8
            for m, w_ref in enumerate((wg, wu)):
                ww = w_ref[pl.ds(l * 8, 8), :]
                for p, wf in enumerate((ww << 16, ww & HI)):
                    wf = pltpu.bitcast(wf, F32)
                    here = lane - 2 * sub == 16 * (l % 8) + p
                    for c in range(2):
                        val = jnp.sum(wf * xsel[c], axis=1, keepdims=True)
                        pre[m, c] = jnp.where(here, val, pre.get((m, c), np.float32(0)))
            if l % 8 == 7 or l == F // 16 - 1:
                hh = jnp.concatenate([jax.nn.silu(pre.pop((0, c))) * pre.pop((1, c)) for c in range(2)], axis=0)
                hbuf[:, pl.ds(T * 128, 128)] = pltpu.bitcast(hh.astype(BF16), I32)

        def down():
            yy = jnp.dot(pltpu.bitcast(hbuf[:, pl.ds(0, F)], BF16), pltpu.bitcast(wd[...], BF16), preferred_element_type=F32)
            ys = []
            for c, k in enumerate(sel["keys"]):
                kb = jnp.full((1, 128), k & HI, I32)
                rs = jax.nn.sigmoid(pltpu.bitcast(jnp.where(kb < 0, kb ^ np.int32(0x7FFF0000), kb), F32))
                ys.append(jnp.sum(yy[8 * c:8 * c + 8], axis=0, keepdims=True) * jnp.concatenate([rs] * NT, axis=1))
            return sel["idx"], ys

        def patch(idx, yy):
            subD = lax.broadcasted_iota(I32, (16, D), 0)
            for c, t in enumerate(idx):
                rows = pl.ds(pl.multiple_of((t >> 4) << 3, 8), 8)
                blk = pltpu.bitcast(ax[rows, :], BF16).astype(F32)
                blk = jnp.where(subD == (t & 15), blk + yy[c], blk)
                ax[rows, :] = pltpu.bitcast(blk.astype(BF16), I32)

        cp_o = [pltpu.make_async_copy(out_s.at[pl.ds(r0 // 2, n // 2)], out_h.at[pl.ds(r0 // 2, n // 2)], so.at[i])
                for i, (r0, n) in enumerate(outs)]

        def out_block(r0, n):
            assert att_done >= r0 + n
            rows = pl.ds(r0 // 2, n // 2)
            a = jnp.dot(pltpu.bitcast(o_s[rows, :], BF16), pltpu.bitcast(wop[...], BF16), preferred_element_type=F32)
            b = pltpu.bitcast(ax[rows, :], BF16).astype(F32)
            g = g_rep[pl.ds(r0, n), :]
            g = jnp.concatenate([g] * NT, axis=1)
            out_s[rows, :] = pltpu.bitcast((b + g * (a - b)).astype(BF16), I32)

        for j in range(NT):
            qkv[NT + j, pl.ds(0, HALO), :] = jnp.zeros((HALO, 128), F32)
        att = attn_steps()
        need = next(att)
        pending = []

        def run_aux(r):
            if "rt" in r:
                for g in range(r["rt"][0] // 16, r["rt"][1] // 16):
                    router(g)
            if r.get("select"):
                select()
            for l in () if r.get("select") else r.get("xp", ()):
                gate_up(l)
            if "gx" in r:
                gc = [g_s[0], g_s[1]]
                for m in range(r["gx"][0] // 8, r["gx"][1] // 8):
                    g_rep[pl.ds(m * 8, 8), :] = jnp.broadcast_to(gc[m // 128][:, m % 128:m % 128 + 1], (8, 128))
            for j in r.get("wo", ()):
                for d in range(DH // 2):
                    wo_gather(j, d)

        for k, r in enumerate(regions):
            with scope(str(k)):
                for d in r.get("wait", []):
                    for c in cps[d]:
                        c.wait()
                if r.get("name") not in merge:
                    pl.semaphore_signal(sbar, 1)
                    pl.semaphore_wait(sbar, 1)
                if r.get("patch"):
                    patch(*res)
                for p in r.get("perm", []):
                    permute_chunk(*p)
                for fn in pending:
                    fn()
                pending = []
                for k0, k1, ra, rb in r.get("kmm", ()):
                    for a in range(ra, rb, kmr):
                        y = jnp.dot(pltpu.bitcast(ax[pl.ds(a // 2, kmr // 2), k0 * 128:k1 * 128], BF16),
                                    pltpu.bitcast(wp[k0 * 64:k1 * 64, D:2 * D], BF16), preferred_element_type=F32)
                        for j in range(NT):
                            dst = (NT + j, pl.ds(HALO + a, kmr), slice(None))
                            yj = y[:, j * 128:(j + 1) * 128]
                            qkv[dst] = qkv[dst] + yj if k0 else yj
                if auxpos == "start":
                    run_aux(r)
                mms = list(r.get("mm", []))
                if defer and mms and k + 1 < len(regions) and not r.get("halo"):
                    s_, r0, n = mms.pop()
                    if n > defer:
                        mms.append((s_, r0, n - defer))
                    for m in mms:
                        qkv_mm(*m)()
                    pending.append(qkv_mm(s_, r0 + n - min(n, defer), min(n, defer)))
                else:
                    for m in mms:
                        qkv_mm(*m)()
                if r.get("halo"):
                    for j in range(NT):
                        qkv[2 * NT + j, pl.ds(0, HALO), :] = jnp.broadcast_to(qkv[2 * NT + j, pl.ds(HALO, 1), :], (HALO, 128))
                late = [o for o in r.get("out", []) if att_done < sum(o)]
                for o in r.get("out", []):
                    if o not in late:
                        out_block(*o)
                if auxpos == "mid":
                    run_aux(r)
                while need is not None and need <= r.get("att", 0):
                    need = next(att, None)
                for l in r.get("xp", ()) if r.get("select") else ():
                    gate_up(l)
                for o in late:
                    out_block(*o)
                if auxpos == "end":
                    run_aux(r)
                if r.get("ffn"):
                    res = down()
                for o in r.get("out", []):
                    cp_o[outs.index(o)].start()
        with scope("tail"):
            for c in cp_o:
                c.wait()

    def f(A_x, A_wqkv, A_wo, B_x, B_w_r, B_w_gate, B_w_up, B_w_down, gate_w):
        hbm = pl.BlockSpec(memory_space=pltpu.HBM)
        vm = pl.BlockSpec(memory_space=pltpu.VMEM)
        out = pl.pallas_call(
            kern,
            out_shape=jax.ShapeDtypeStruct((S, D), BF16),
            in_specs=[hbm] * 8,
            out_specs=hbm,
            scratch_shapes=[
                pltpu.VMEM((S // 2, D), I32),
                pltpu.VMEM((3, D // 2, D), I32), pltpu.VMEM((D // 2, 3 * D), I32),
                pltpu.VMEM((NT, D // 2, 128), I32), pltpu.VMEM((D // 2, D), I32),
                pltpu.VMEM((F // 2, D), I32), pltpu.VMEM((F // 2, D), I32), pltpu.VMEM((F // 2, D), I32),
                pltpu.VMEM((2, 8, D), F32), pltpu.VMEM((8, 1792), I32),
                pltpu.VMEM((3 * NT, HALO + ring, 128), F32),
                pltpu.VMEM((S // 2, D), I32), pltpu.VMEM((S // 2, D), I32),
                pltpu.VMEM((2, 8, 128), F32), pltpu.VMEM((S, 128), F32), pltpu.VMEM((D,), BF16), pltpu.VMEM((D,), BF16),
                pltpu.SemaphoreType.DMA((len(dma) + 7,)), pltpu.SemaphoreType.DMA((len(outs),)), pltpu.SemaphoreType.REGULAR,
            ],
            compiler_params=pltpu.CompilerParams(vmem_limit_bytes=100 * 2**20, flags=flags),
        )(A_x.reshape(S, D), A_wqkv, A_wo, B_w_r, B_w_gate.T, B_w_up.T, B_w_down, gate_w)
        return out.reshape(1, S, D)
    return f


_impl = make(**dict())


@jax.jit
def pallas_gated_mix__sliding_local_dilated__moe_arch_mod__prompt_kernel(
    A_x, A_wqkv, A_wo, B_x, B_w_r, B_w_gate, B_w_up, B_w_down, gate_w
):
    return _impl(A_x, A_wqkv, A_wo, B_x, B_w_r, B_w_gate, B_w_up, B_w_down, gate_w)
```

```python
import jax
import jax.numpy as jnp
import numpy as np
from jax import lax
from jax.experimental import pallas as pl
from jax.experimental.pallas import tpu as pltpu

S, D, H, DH, W, DIL, F = 2048, 640, 32, 20, 8, 2, 1728
NT = D // 128
HALO = 16
MM = 128
Q, K, V = 0, 1, 2
F32, BF16, I32 = jnp.float32, jnp.bfloat16, jnp.int32
HI = np.int32(-65536)
INT_MIN = np.int32(-2**31)
Q_SCALE = np.float32(DH ** -0.5 * np.log2(np.e))
MASKED = np.float32(-1e9 * np.log2(np.e))


def _plan():
    xa, wa, xb, wb = ("xc", 0, 2), ("w", K, 0, 2), ("xc", 2, NT), ("w", K, 2, NT)
    wq, wv, x1, x2 = ("w", Q, 0, NT), ("w", V, 0, NT), ("x", 512, 896), ("x", 896, S)
    dma = [xa, wa, xb, wb, ("vec",), wq, wv, x1, x2, ("wo",), ("gu",), ("down",)]

    def mm(*blocks):
        return [(s, r0 + a) for s, r0 in blocks for a in range(0, 256, MM)]

    def stage(r0, att, **kw):
        return dict(mm=mm((K, r0), (Q, r0), (V, r0)), att=att, **kw)

    return dma, [
        dict(wait=[xa, wa], perm=wa[1:], kmm=[(0, 2, 0, 512)]),
        dict(wait=[xb, wb, ("vec",)], perm=wb[1:], kmm=[(2, NT, 0, 384)], route=(0, 256)),
        dict(wait=[wq], perm=wq[1:], kmm=[(2, NT, 384, 512)], route=(256, 512), mm=mm((Q, 0))),
        dict(wait=[wv, x1], perm=wv[1:], route=(512, 896), mm=mm((Q, 256), (V, 0), (V, 256)), halo=True),
        stage(512, 256, wait=[x2, ("wo",)], route=(896, 1536)),
        stage(768, 512, route=(1536, S), fused=True),
        stage(1024, 816, select=True),
        stage(1280, 1008, wait=[("gu",)], gate_up=(0, 54), perm_wo=True),
        stage(1536, 1200, wait=[("down",)], gate_up=(54, F // 16)),
        stage(1792, 1504, gates=(0, 768), down=True, fused=True),
        dict(patch=True, gates=(768, 1536), out=[(0, 256), (256, 256), (512, 256)], att=1776),
        dict(gates=(1536, 1920), out=[(768, 256), (1024, 256), (1280, 256)], att=S),
        dict(gates=(1920, S), out=[(1536, 256), (1792, 128)]),
        dict(out=[(1920, 128)]),
    ]


_DMA, _REGIONS = _plan()
_OUTS = [o for r in _REGIONS for o in r.get("out", ())]
_IN_SEMS = len(_DMA) + NT + 1


def _tree(f, xs):
    while len(xs) > 1:
        xs = [f(xs[k], xs[k + 1]) if k + 1 < len(xs) else xs[k] for k in range(0, len(xs), 2)]
    return xs[0]


def _rows(r0, n):
    return pl.ds(r0 // 2, n // 2)


def _bf16(words):
    return pltpu.bitcast(words, BF16)


def _words(x):
    return pltpu.bitcast(x.astype(BF16), I32)


def _ordered(bits):
    return jnp.where(bits < 0, bits ^ np.int32(0x7FFF0000), bits)


def _kernel(x_hbm, wqkv_hbm, wo_hbm, wr_hbm, wg_hbm, wu_hbm, wd_hbm, gw_hbm, out_hbm,
            x, wraw, wp, wo_raw, wop, wg, wu, wd, wr, gw,
            qkv, att_out, out, gate, gate_rep, xsel, hidden, in_sem, out_sem, barrier):
    x_h, wqkv_h, out_h = (r.bitcast(I32) for r in (x_hbm, wqkv_hbm, out_hbm))

    copies, n_sem = {}, 0
    for d in _DMA:
        if d[0] == "w":
            rows = _rows(d[2] * 128, (d[3] - d[2]) * 128)
            pairs = [(wqkv_h.at[rows, pl.ds(d[1] * D, D)], wraw.at[d[1], rows])]
        elif d[0] == "xc":
            blk = (_rows(0, 512), pl.ds(d[1] * 128, (d[2] - d[1]) * 128))
            pairs = [(x_h.at[blk], x.at[blk])]
        elif d[0] == "x":
            rows = _rows(d[1], d[2] - d[1])
            pairs = [(x_h.at[rows], x.at[rows])]
        elif d[0] == "vec":
            pairs = [(wr_hbm, wr), (gw_hbm, gw)]
        elif d[0] == "wo":
            pairs = [(wo_hbm.bitcast(I32).at[:, pl.ds(j * 128, 128)], wo_raw.at[j]) for j in range(NT)]
        elif d[0] == "gu":
            pairs = [(wg_hbm.bitcast(I32), wg), (wu_hbm.bitcast(I32), wu)]
        else:
            pairs = [(wd_hbm.bitcast(I32), wd)]
        copies[d] = [pltpu.make_async_copy(a, b, in_sem.at[n_sem + k]) for k, (a, b) in enumerate(pairs)]
        n_sem += len(pairs)
        for c in copies[d]:
            c.start()
    out_copies = {o: pltpu.make_async_copy(out.at[_rows(*o)], out_h.at[_rows(*o)], out_sem.at[k])
                  for k, o in enumerate(_OUTS)}

    lane = lax.broadcasted_iota(I32, (8, 128), 1)
    sub = lax.broadcasted_iota(I32, (8, 128), 0)

    def permute_wqkv(s, k0, k1):
        for jp in range(NT):
            src = (DH * (lane & 31) + 4 * jp + (lane >> 5)) & 127
            tile = (DH * ((13 * ((lane >> 2) - jp)) & 31) + 4 * jp + (lane & 3)) >> 7
            for r in range(k0 * 8, k1 * 8):
                rows = pl.ds(r * 8, 8)
                acc = wraw[s, rows, pl.ds(0, 128)]
                for j in range(1, NT):
                    acc = jnp.where(tile == j, wraw[s, rows, pl.ds(j * 128, 128)], acc)
                wp[rows, pl.ds(s * D + jp * 128, 128)] = jnp.take_along_axis(acc, src, axis=1)

    def permute_wo():
        for j in range(NT):
            cols = pl.ds(j * 128, 128)
            for i in range(DH // 2):
                even = wo_raw[j, pl.ds(i, H // 2, stride=DH), :]
                odd = wo_raw[j, pl.ds(DH // 2 + i, H // 2, stride=DH), :]
                wop[pl.ds(i * 32, 16), cols] = (even & 0xFFFF) | (odd << 16)
                wop[pl.ds(i * 32 + 16, 16), cols] = lax.shift_right_logical(even, 16) | (odd & HI)

    def project(s, r0, k0=0, k1=NT):
        y = jnp.dot(_bf16(x[_rows(r0, MM), k0 * 128:k1 * 128]), _bf16(wp[k0 * 64:k1 * 64, s * D:(s + 1) * D]),
                    preferred_element_type=F32)
        if s == Q:
            y = y * Q_SCALE
        for j in range(NT):
            dst = (s * NT + j, pl.ds(HALO + r0, MM), slice(None))
            yj = y[:, j * 128:(j + 1) * 128]
            qkv[dst] = qkv[dst] + yj if k0 else yj

    att_done = 0

    def attention():
        nonlocal att_done
        lag, n = 6, S // 8 * W
        half, quarter, logit, weight, acc = {}, {}, {}, {}, [None] * NT
        for t in range(n + 3 * lag + W):
            yield min(S, (t // W + 1) * 8)
            if t < n:
                g, w = divmod(t, W)
                if w == 0:
                    q = [qkv[Q * NT + j, pl.ds(HALO + g * 8, 8), :] for j in range(NT)]
                rows = pl.ds(HALO + g * 8 - DIL * w, 8)
                a = q[0] * qkv[K * NT, rows, :]
                for j in range(1, NT):
                    a = a + q[j] * qkv[K * NT + j, rows, :]
                half[t] = (a, pltpu.roll(a, 64, 1))
            u = t - lag
            if 0 <= u < n:
                a, b = half.pop(u)
                a = a + b
                quarter[u] = (a, pltpu.roll(a, 32, 1))
            u = t - 2 * lag
            if 0 <= u < n:
                g, w = divmod(u, W)
                a, b = quarter.pop(u)
                a = a + b
                if g * 8 < DIL * w:
                    a = jnp.where(sub + g * 8 >= DIL * w, a, MASKED)
                logit[u] = a
                if w == W - 1:
                    row = [logit.pop(g * W + k) for k in range(W)]
                    top = _tree(jnp.maximum, row)
                    for k in range(W):
                        weight[g * W + k] = jnp.exp2(row[k] - top)
            u = t - 3 * lag - (W - 1)
            if 0 <= u < n:
                g, w = divmod(u, W)
                if w == 0:
                    den = _tree(jnp.add, [weight[g * W + k] for k in range(W)])
                    inv = pl.reciprocal(den, approx=True)
                if w == W // 2:
                    inv = inv * (2.0 - den * inv)
                e = weight.pop(u)
                rows = pl.ds(HALO + g * 8 - DIL * w, 8)
                for j in range(NT):
                    p = e * qkv[V * NT + j, rows, :]
                    acc[j] = p if w == 0 else acc[j] + p
                if w == W - 1:
                    o = [a * inv for a in acc]
                    if g % 2 == 0:
                        held = o
                    else:
                        for j in range(NT):
                            att_out[_rows((g - 1) * 8, 16), pl.ds(j * 128, 128)] = _words(
                                jnp.concatenate([held[j], o[j]], axis=0))
                        att_done = (g + 1) * 8

    score = [jnp.zeros((8, 128), F32)] * 2
    gate_logit = list(score)
    vecs, picked = [], {}

    def route(r0, r1):
        if not vecs:
            vecs.extend(jnp.broadcast_to(v[...].astype(F32).reshape(1, D), (8, D)) for v in (wr, gw))
        for g in range(r0 // 16, r1 // 16):
            xf = _bf16(x[_rows(g * 16, 16), :]).astype(F32)
            for p in range(2):
                c, l = divmod(2 * g + p, 128)
                for dst, vec in zip((score, gate_logit), vecs):
                    val = jnp.sum(xf[8 * p:8 * p + 8] * vec, axis=1, keepdims=True)
                    dst[c] = jnp.where(lane == l, val, dst[c])

    def token_group(t):
        return pl.ds(pl.multiple_of((t >> 4) << 3, 8), 8), lax.broadcasted_iota(I32, (16, D), 0) == (t & 15)

    def select():
        keys = []
        for c in range(2):
            gate[c] = jax.nn.sigmoid(gate_logit[c])
        for c in range(2):
            r = score[c].astype(BF16).astype(F32)
            r = jnp.where(r == 0, np.float32(0), r)
            key = jnp.where(r != r, INT_MIN, _ordered(pltpu.bitcast(r, I32)))
            keys.append(key | (S - 1 - (1024 * c + 8 * lane + sub)))
        k1 = jnp.max(jnp.maximum(*keys))
        k2 = jnp.max(jnp.maximum(*[jnp.where(k == k1, INT_MIN, k) for k in keys]))
        picked["keys"] = (k1, k2)
        picked["rows"] = [S - 1 - (k & (S - 1)) for k in (k1, k2)]
        for c, t in enumerate(picked["rows"]):
            rows, here = token_group(t)
            row = jnp.sum(jnp.where(here, _bf16(x[rows, :]).astype(F32), 0.0), axis=0, keepdims=True)
            xsel[c] = jnp.broadcast_to(row, (8, D))

    pre = {}

    def gate_up(l):
        for m, w_ref in enumerate((wg, wu)):
            ww = w_ref[pl.ds(l * 8, 8), :]
            for p, wf in enumerate((ww << 16, ww & HI)):
                here = lane - 2 * sub == 16 * (l % 8) + p
                for c in range(2):
                    val = jnp.sum(pltpu.bitcast(wf, F32) * xsel[c], axis=1, keepdims=True)
                    pre[m, c] = jnp.where(here, val, pre.get((m, c), np.float32(0)))
        if l % 8 == 7 or l == F // 16 - 1:
            h = [jax.nn.silu(pre.pop((0, c))) * pre.pop((1, c)) for c in range(2)]
            hidden[:, pl.ds(l // 8 * 128, 128)] = _words(jnp.concatenate(h, axis=0))

    def down():
        y = jnp.dot(_bf16(hidden[:, pl.ds(0, F)]), _bf16(wd[...]), preferred_element_type=F32)
        picked["update"] = []
        for c, k in enumerate(picked["keys"]):
            r = jax.nn.sigmoid(pltpu.bitcast(_ordered(jnp.full((1, 128), k & HI, I32)), F32))
            yc = jnp.sum(y[8 * c:8 * c + 8], axis=0, keepdims=True)
            picked["update"].append(yc * jnp.concatenate([r] * NT, axis=1))

    def patch():
        for t, upd in zip(picked["rows"], picked["update"]):
            rows, here = token_group(t)
            blk = _bf16(x[rows, :]).astype(F32)
            x[rows, :] = _words(jnp.where(here, blk + upd, blk))

    def mix(r0, n):
        rows = _rows(r0, n)
        a = jnp.dot(_bf16(att_out[rows, :]), _bf16(wop[...]), preferred_element_type=F32)
        b = _bf16(x[rows, :]).astype(F32)
        g = jnp.concatenate([gate_rep[pl.ds(r0, n), :]] * NT, axis=1)
        out[rows, :] = _words(b + g * (a - b))

    for j in range(NT):
        qkv[K * NT + j, pl.ds(0, HALO), :] = jnp.zeros((HALO, 128), F32)
    steps = attention()
    need = next(steps)
    for r in _REGIONS:
        for d in r.get("wait", ()):
            for c in copies[d]:
                c.wait()
        if not r.get("fused"):
            pl.semaphore_signal(barrier, 1)
            pl.semaphore_wait(barrier, 1)
        if r.get("patch"):
            patch()
        if "perm" in r:
            permute_wqkv(*r["perm"])
        for k0, k1, r0, r1 in r.get("kmm", ()):
            for a in range(r0, r1, MM):
                project(K, a, k0, k1)
        if "route" in r:
            route(*r["route"])
        if r.get("select"):
            select()
        for l in range(*r.get("gate_up", (0,))):
            gate_up(l)
        if "gates" in r:
            compact = [gate[0], gate[1]]
            for m in range(r["gates"][0] // 8, r["gates"][1] // 8):
                c, l = divmod(m, 128)
                gate_rep[pl.ds(m * 8, 8), :] = jnp.broadcast_to(compact[c][:, l:l + 1], (8, 128))
        if r.get("perm_wo"):
            permute_wo()
        for s, r0 in r.get("mm", ()):
            project(s, r0)
        if r.get("halo"):
            for j in range(NT):
                first = qkv[V * NT + j, pl.ds(HALO, 1), :]
                qkv[V * NT + j, pl.ds(0, HALO), :] = jnp.broadcast_to(first, (HALO, 128))
        for r0, n in r.get("out", ()):
            assert att_done >= r0 + n
            mix(r0, n)
        while need is not None and need <= r.get("att", 0):
            need = next(steps, None)
        if r.get("down"):
            down()
        for o in r.get("out", ()):
            out_copies[o].start()
    for o in _OUTS:
        out_copies[o].wait()


@jax.jit
def pallas_gated_mix__sliding_local_dilated__moe_arch_mod__prompt_kernel(
    A_x: jax.Array,
    A_wqkv: jax.Array,
    A_wo: jax.Array,
    B_x: jax.Array,
    B_w_r: jax.Array,
    B_w_gate: jax.Array,
    B_w_up: jax.Array,
    B_w_down: jax.Array,
    gate_w: jax.Array,
):
    del B_x
    hbm = pl.BlockSpec(memory_space=pltpu.HBM)
    out = pl.pallas_call(
        _kernel,
        out_shape=jax.ShapeDtypeStruct((S, D), BF16),
        in_specs=[hbm] * 8,
        out_specs=hbm,
        scratch_shapes=[
            pltpu.VMEM((S // 2, D), I32),
            pltpu.VMEM((3, D // 2, D), I32),
            pltpu.VMEM((D // 2, 3 * D), I32),
            pltpu.VMEM((NT, D // 2, 128), I32),
            pltpu.VMEM((D // 2, D), I32),
            pltpu.VMEM((F // 2, D), I32),
            pltpu.VMEM((F // 2, D), I32),
            pltpu.VMEM((F // 2, D), I32),
            pltpu.VMEM((D,), BF16),
            pltpu.VMEM((D,), BF16),
            pltpu.VMEM((3 * NT, HALO + S, 128), F32),
            pltpu.VMEM((S // 2, D), I32),
            pltpu.VMEM((S // 2, D), I32),
            pltpu.VMEM((2, 8, 128), F32),
            pltpu.VMEM((S, 128), F32),
            pltpu.VMEM((2, 8, D), F32),
            pltpu.VMEM((8, pl.cdiv(F, 128) * 128), I32),
            pltpu.SemaphoreType.DMA((_IN_SEMS,)),
            pltpu.SemaphoreType.DMA((len(_OUTS),)),
            pltpu.SemaphoreType.REGULAR,
        ],
        compiler_params=pltpu.CompilerParams(vmem_limit_bytes=64 * 2**20),
    )(A_x.reshape(S, D), A_wqkv, A_wo, B_w_r, B_w_gate.T, B_w_up.T, B_w_down, gate_w)
    return out.reshape(1, S, D)
```

```python
import jax
import jax.numpy as jnp
import numpy as np
from jax import lax
from jax.experimental import pallas as pl
from jax.experimental.pallas import tpu as pltpu

S, D, H, DH, W, DIL, F = 2048, 640, 32, 20, 8, 2, 1728
NT = D // 128
HALO = 16
MM = 128
Q, K, V = 0, 1, 2
F32, BF16, I32 = jnp.float32, jnp.bfloat16, jnp.int32
HI = np.int32(-65536)
INT_MIN = np.int32(-2**31)
Q_SCALE = np.float32(DH ** -0.5 * np.log2(np.e))
MASKED = np.float32(-1e9 * np.log2(np.e))


def _plan():
    xa, wa, xb, wb = ("xc", 0, 2), ("w", K, 0, 2), ("xc", 2, NT), ("w", K, 2, NT)
    wq, wv, x1, x2 = ("w", Q, 0, NT), ("w", V, 0, NT), ("x", 512, 896), ("x", 896, S)
    dma = [wa, xa, wb, xb, ("vec",), wq, wv, x1, x2, ("wo",), ("gu",), ("down",)]

    def mm(*blocks):
        return [(s, r0 + a) for s, r0 in blocks for a in range(0, 256, MM)]

    def stage(r0, att, **kw):
        return dict(mm=mm((V, r0), (Q, r0), (K, r0)), att=att, **kw)

    return dma, [
        dict(wait=[wa], perm=wa[1:]),
        dict(wait=[xa], kmm=[(0, 2, 0, 512)]),
        dict(wait=[wb], perm=wb[1:]),
        dict(wait=[xb, ("vec",)], kmm=[(2, NT, 0, 384)], route=(0, 256)),
        dict(wait=[wq], perm=wq[1:], kmm=[(2, NT, 384, 512)], route=(256, 512), mm=mm((Q, 0))),
        dict(wait=[wv, x1], perm=wv[1:], route=(512, 896), mm=mm((Q, 256), (V, 0), (V, 256)), halo=True),
        stage(512, 256, wait=[x2, ("wo",)], route=(896, 1536)),
        stage(768, 512, route=(1536, S), fused=True),
        stage(1024, 816, select=True),
        stage(1280, 1008, wait=[("gu",)], gate_up=(0, 54), perm_wo=True),
        stage(1536, 1200, wait=[("down",)], gate_up=(54, F // 16)),
        stage(1792, 1504, gates=(0, 768), down=True, fused=True),
        dict(patch=True, gates=(768, 1536), out=[(0, 256), (256, 256), (512, 256)], att=1776),
        dict(gates=(1536, 1920), out=[(768, 256), (1024, 256), (1280, 256)], att=S),
        dict(gates=(1920, S), out=[(1536, 256), (1792, 128)]),
        dict(out=[(1920, 128)]),
    ]


_DMA, _REGIONS = _plan()
_OUTS = [o for r in _REGIONS for o in r.get("out", ())]
_IN_SEMS = len(_DMA) + NT + 1


def _tree(f, xs):
    while len(xs) > 1:
        xs = [f(xs[k], xs[k + 1]) if k + 1 < len(xs) else xs[k] for k in range(0, len(xs), 2)]
    return xs[0]


def _rows(r0, n):
    return pl.ds(r0 // 2, n // 2)


def _bf16(words):
    return pltpu.bitcast(words, BF16)


def _words(x):
    return pltpu.bitcast(x.astype(BF16), I32)


def _ordered(bits):
    return jnp.where(bits < 0, bits ^ np.int32(0x7FFF0000), bits)


def _kernel(x_hbm, wqkv_hbm, wo_hbm, wr_hbm, wg_hbm, wu_hbm, wd_hbm, gw_hbm, out_hbm,
            x, wraw, wp, wo_raw, wop, wg, wu, wd, wr, gw,
            qkv, att_out, out, gate, gate_rep, xsel, hidden, in_sem, out_sem, barrier):
    x_h, wqkv_h, out_h = (r.bitcast(I32) for r in (x_hbm, wqkv_hbm, out_hbm))

    copies, n_sem = {}, 0
    for d in _DMA:
        if d[0] == "w":
            rows = _rows(d[2] * 128, (d[3] - d[2]) * 128)
            pairs = [(wqkv_h.at[rows, pl.ds(d[1] * D, D)], wraw.at[d[1], rows])]
        elif d[0] == "xc":
            blk = (_rows(0, 512), pl.ds(d[1] * 128, (d[2] - d[1]) * 128))
            pairs = [(x_h.at[blk], x.at[blk])]
        elif d[0] == "x":
            rows = _rows(d[1], d[2] - d[1])
            pairs = [(x_h.at[rows], x.at[rows])]
        elif d[0] == "vec":
            pairs = [(wr_hbm, wr), (gw_hbm, gw)]
        elif d[0] == "wo":
            pairs = [(wo_hbm.bitcast(I32).at[:, pl.ds(j * 128, 128)], wo_raw.at[j]) for j in range(NT)]
        elif d[0] == "gu":
            pairs = [(wg_hbm.bitcast(I32), wg), (wu_hbm.bitcast(I32), wu)]
        else:
            pairs = [(wd_hbm.bitcast(I32), wd)]
        copies[d] = [pltpu.make_async_copy(a, b, in_sem.at[n_sem + k]) for k, (a, b) in enumerate(pairs)]
        n_sem += len(pairs)
        for c in copies[d]:
            c.start()
    out_copies = {o: pltpu.make_async_copy(out.at[_rows(*o)], out_h.at[_rows(*o)], out_sem.at[k])
                  for k, o in enumerate(_OUTS)}

    lane = lax.broadcasted_iota(I32, (8, 128), 1)
    sub = lax.broadcasted_iota(I32, (8, 128), 0)

    def permute_wqkv(s, k0, k1):
        for jp in range(NT):
            src = (DH * (lane & 31) + 4 * jp + (lane >> 5)) & 127
            tile = (DH * ((13 * ((lane >> 2) - jp)) & 31) + 4 * jp + (lane & 3)) >> 7
            for r in range(k0 * 8, k1 * 8):
                rows = pl.ds(r * 8, 8)
                acc = wraw[s, rows, pl.ds(0, 128)]
                for j in range(1, NT):
                    acc = jnp.where(tile == j, wraw[s, rows, pl.ds(j * 128, 128)], acc)
                wp[rows, pl.ds(s * D + jp * 128, 128)] = jnp.take_along_axis(acc, src, axis=1)

    def permute_wo():
        for j in range(NT):
            cols = pl.ds(j * 128, 128)
            for i in range(DH // 2):
                even = wo_raw[j, pl.ds(i, H // 2, stride=DH), :]
                odd = wo_raw[j, pl.ds(DH // 2 + i, H // 2, stride=DH), :]
                wop[pl.ds(i * 32, 16), cols] = (even & 0xFFFF) | (odd << 16)
                wop[pl.ds(i * 32 + 16, 16), cols] = lax.shift_right_logical(even, 16) | (odd & HI)

    def project(s, r0, k0=0, k1=NT):
        y = jnp.dot(_bf16(x[_rows(r0, MM), k0 * 128:k1 * 128]), _bf16(wp[k0 * 64:k1 * 64, s * D:(s + 1) * D]),
                    preferred_element_type=F32)
        if s == Q:
            y = y * Q_SCALE
        for j in range(NT):
            dst = (s * NT + j, pl.ds(HALO + r0, MM), slice(None))
            yj = y[:, j * 128:(j + 1) * 128]
            qkv[dst] = qkv[dst] + yj if k0 else yj

    att_done = 0

    def attention():
        nonlocal att_done
        lags, n = (6, 12, 18), S // 8 * W
        half, quarter, logit, weight, acc = {}, {}, {}, {}, [None] * NT
        for t in range(n + lags[2] + W):
            yield min(S, (t // W + 1) * 8)
            if t < n:
                g, w = divmod(t, W)
                if w == 0:
                    q = [qkv[Q * NT + j, pl.ds(HALO + g * 8, 8), :] for j in range(NT)]
                rows = pl.ds(HALO + g * 8 - DIL * w, 8)
                a = q[0] * qkv[K * NT, rows, :]
                for j in range(1, NT):
                    a = a + q[j] * qkv[K * NT + j, rows, :]
                half[t] = (a, pltpu.roll(a, 64, 1))
            u = t - lags[0]
            if 0 <= u < n:
                a, b = half.pop(u)
                a = a + b
                quarter[u] = (a, pltpu.roll(a, 32, 1))
            u = t - lags[1]
            if 0 <= u < n:
                g, w = divmod(u, W)
                a, b = quarter.pop(u)
                a = a + b
                if g * 8 < DIL * w:
                    a = jnp.where(sub + g * 8 >= DIL * w, a, MASKED)
                logit[u] = a
                if w == W - 1:
                    row = [logit.pop(g * W + k) for k in range(W)]
                    top = _tree(jnp.maximum, row)
                    for k in range(W):
                        weight[g * W + k] = jnp.exp2(row[k] - top)
            u = t - lags[2] - (W - 1)
            if 0 <= u < n:
                g, w = divmod(u, W)
                if w == 0:
                    den = _tree(jnp.add, [weight[g * W + k] for k in range(W)])
                    inv = pl.reciprocal(den, approx=True)
                if w == W // 2:
                    inv = inv * (2.0 - den * inv)
                e = weight.pop(u)
                rows = pl.ds(HALO + g * 8 - DIL * w, 8)
                for j in range(NT):
                    p = e * qkv[V * NT + j, rows, :]
                    acc[j] = p if w == 0 else acc[j] + p
                if w == W - 1:
                    o = [a * inv for a in acc]
                    if g % 2 == 0:
                        held = o
                    else:
                        for j in range(NT):
                            att_out[_rows((g - 1) * 8, 16), pl.ds(j * 128, 128)] = _words(
                                jnp.concatenate([held[j], o[j]], axis=0))
                        att_done = (g + 1) * 8

    score = [jnp.zeros((8, 128), F32)] * 2
    gate_logit = list(score)
    vecs, picked = [], {}

    def route(r0, r1):
        if not vecs:
            vecs.extend(jnp.broadcast_to(v[...].astype(F32).reshape(1, D), (8, D)) for v in (wr, gw))
        for g in range(r0 // 16, r1 // 16):
            xf = _bf16(x[_rows(g * 16, 16), :]).astype(F32)
            for p in range(2):
                c, l = divmod(2 * g + p, 128)
                for dst, vec in zip((score, gate_logit), vecs):
                    val = jnp.sum(xf[8 * p:8 * p + 8] * vec, axis=1, keepdims=True)
                    dst[c] = jnp.where(lane == l, val, dst[c])

    def token_group(t):
        return pl.ds(pl.multiple_of((t >> 4) << 3, 8), 8), lax.broadcasted_iota(I32, (16, D), 0) == (t & 15)

    def select():
        keys = []
        for c in range(2):
            gate[c] = jax.nn.sigmoid(gate_logit[c])
        for c in range(2):
            r = score[c].astype(BF16).astype(F32)
            r = jnp.where(r == 0, np.float32(0), r)
            key = jnp.where(r != r, INT_MIN, _ordered(pltpu.bitcast(r, I32)))
            keys.append(key | (S - 1 - (1024 * c + 8 * lane + sub)))
        k1 = jnp.max(jnp.maximum(*keys))
        k2 = jnp.max(jnp.maximum(*[jnp.where(k == k1, INT_MIN, k) for k in keys]))
        picked["keys"] = (k1, k2)
        picked["rows"] = [S - 1 - (k & (S - 1)) for k in (k1, k2)]
        for c, t in enumerate(picked["rows"]):
            rows, here = token_group(t)
            row = jnp.sum(jnp.where(here, _bf16(x[rows, :]).astype(F32), 0.0), axis=0, keepdims=True)
            xsel[c] = jnp.broadcast_to(row, (8, D))

    pre = {}

    def gate_up(l):
        for m, w_ref in enumerate((wg, wu)):
            ww = w_ref[pl.ds(l * 8, 8), :]
            for p, wf in enumerate((ww << 16, ww & HI)):
                here = lane - 2 * sub == 16 * (l % 8) + p
                for c in range(2):
                    val = jnp.sum(pltpu.bitcast(wf, F32) * xsel[c], axis=1, keepdims=True)
                    pre[m, c] = jnp.where(here, val, pre.get((m, c), np.float32(0)))
        if l % 8 == 7 or l == F // 16 - 1:
            h = [jax.nn.silu(pre.pop((0, c))) * pre.pop((1, c)) for c in range(2)]
            hidden[:, pl.ds(l // 8 * 128, 128)] = _words(jnp.concatenate(h, axis=0))

    def down():
        y = jnp.dot(_bf16(hidden[:, pl.ds(0, F)]), _bf16(wd[...]), preferred_element_type=F32)
        picked["update"] = []
        for c, k in enumerate(picked["keys"]):
            r = jax.nn.sigmoid(pltpu.bitcast(_ordered(jnp.full((1, 128), k & HI, I32)), F32))
            yc = jnp.sum(y[8 * c:8 * c + 8], axis=0, keepdims=True)
            picked["update"].append(yc * jnp.concatenate([r] * NT, axis=1))

    def patch():
        for t, upd in zip(picked["rows"], picked["update"]):
            rows, here = token_group(t)
            blk = _bf16(x[rows, :]).astype(F32)
            x[rows, :] = _words(jnp.where(here, blk + upd, blk))

    def mix(r0, n):
        rows = _rows(r0, n)
        a = jnp.dot(_bf16(att_out[rows, :]), _bf16(wop[...]), preferred_element_type=F32)
        b = _bf16(x[rows, :]).astype(F32)
        g = jnp.concatenate([gate_rep[pl.ds(r0, n), :]] * NT, axis=1)
        out[rows, :] = _words(b + g * (a - b))

    for j in range(NT):
        qkv[K * NT + j, pl.ds(0, HALO), :] = jnp.zeros((HALO, 128), F32)
    steps = attention()
    need = next(steps)
    for r in _REGIONS:
        for d in r.get("wait", ()):
            for c in copies[d]:
                c.wait()
        if not r.get("fused") and not r.get("wait"):
            pl.semaphore_signal(barrier, 1)
            pl.semaphore_wait(barrier, 1)
        if r.get("patch"):
            patch()
        if "perm" in r:
            permute_wqkv(*r["perm"])
        for k0, k1, r0, r1 in r.get("kmm", ()):
            for a in range(r0, r1, MM):
                project(K, a, k0, k1)
        if "route" in r:
            route(*r["route"])
        if r.get("select"):
            select()
        for l in range(*r.get("gate_up", (0,))):
            gate_up(l)
        if "gates" in r:
            compact = [gate[0], gate[1]]
            for m in range(r["gates"][0] // 8, r["gates"][1] // 8):
                c, l = divmod(m, 128)
                gate_rep[pl.ds(m * 8, 8), :] = jnp.broadcast_to(compact[c][:, l:l + 1], (8, 128))
        if r.get("perm_wo"):
            permute_wo()
        for s, r0 in r.get("mm", ()):
            project(s, r0)
        if r.get("halo"):
            for j in range(NT):
                first = qkv[V * NT + j, pl.ds(HALO, 1), :]
                qkv[V * NT + j, pl.ds(0, HALO), :] = jnp.broadcast_to(first, (HALO, 128))
        for r0, n in r.get("out", ()):
            assert att_done >= r0 + n
            mix(r0, n)
        while need is not None and need <= r.get("att", 0):
            need = next(steps, None)
        if r.get("down"):
            down()
        for o in r.get("out", ()):
            out_copies[o].start()
    for o in _OUTS:
        out_copies[o].wait()


@jax.jit
def pallas_gated_mix__sliding_local_dilated__moe_arch_mod__prompt_kernel(
    A_x: jax.Array,
    A_wqkv: jax.Array,
    A_wo: jax.Array,
    B_x: jax.Array,
    B_w_r: jax.Array,
    B_w_gate: jax.Array,
    B_w_up: jax.Array,
    B_w_down: jax.Array,
    gate_w: jax.Array,
):
    del B_x
    hbm = pl.BlockSpec(memory_space=pltpu.HBM)
    out = pl.pallas_call(
        _kernel,
        out_shape=jax.ShapeDtypeStruct((S, D), BF16),
        in_specs=[hbm] * 8,
        out_specs=hbm,
        scratch_shapes=[
            pltpu.VMEM((S // 2, D), I32),
            pltpu.VMEM((3, D // 2, D), I32),
            pltpu.VMEM((D // 2, 3 * D), I32),
            pltpu.VMEM((NT, D // 2, 128), I32),
            pltpu.VMEM((D // 2, D), I32),
            pltpu.VMEM((F // 2, D), I32),
            pltpu.VMEM((F // 2, D), I32),
            pltpu.VMEM((F // 2, D), I32),
            pltpu.VMEM((D,), BF16),
            pltpu.VMEM((D,), BF16),
            pltpu.VMEM((3 * NT, HALO + S, 128), F32),
            pltpu.VMEM((S // 2, D), I32),
            pltpu.VMEM((S // 2, D), I32),
            pltpu.VMEM((2, 8, 128), F32),
            pltpu.VMEM((S, 128), F32),
            pltpu.VMEM((2, 8, D), F32),
            pltpu.VMEM((8, pl.cdiv(F, 128) * 128), I32),
            pltpu.SemaphoreType.DMA((_IN_SEMS,)),
            pltpu.SemaphoreType.DMA((len(_OUTS),)),
            pltpu.SemaphoreType.REGULAR,
        ],
        compiler_params=pltpu.CompilerParams(vmem_limit_bytes=64 * 2**20),
    )(A_x.reshape(S, D), A_wqkv, A_wo, B_w_r, B_w_gate.T, B_w_up.T, B_w_down, gate_w)
    return out.reshape(1, S, D)
```

```python
import jax
import jax.numpy as jnp
import numpy as np
from jax import lax
from jax.experimental import pallas as pl
from jax.experimental.pallas import tpu as pltpu

S, D, H, DH, W, DIL, F = 2048, 640, 32, 20, 8, 2, 1728
NT = D // 128
HALO = 16
MM = 128
Q, K, V = 0, 1, 2
F32, BF16, I32 = jnp.float32, jnp.bfloat16, jnp.int32
HI = np.int32(-65536)
INT_MIN = np.int32(-2**31)
Q_SCALE = np.float32(DH ** -0.5 * np.log2(np.e))
MASKED = np.float32(-1e9 * np.log2(np.e))


def _plan():
    xa, wa, xb, wb = ("xc", 0, 2), ("w", K, 0, 2), ("xc", 2, NT), ("w", K, 2, NT)
    wq, wv, x1, x2 = ("w", Q, 0, NT), ("w", V, 0, NT), ("x", 512, 896), ("x", 896, S)
    dma = [wa, xa, wb, xb, ("vec",), wq, wv, x1, x2, ("wo",), ("gu",), ("down",)]

    def mm(*blocks):
        return [(s, r0 + a) for s, r0 in blocks for a in range(0, 256, MM)]

    def stage(r0, att, **kw):
        return dict(mm=mm((V, r0), (Q, r0), (K, r0)), att=att, **kw)

    return dma, [
        dict(wait=[wa], perm=wa[1:]),
        dict(wait=[xa], kmm=[(0, 2, 0, 512)]),
        dict(wait=[wb], perm=wb[1:]),
        dict(wait=[xb, ("vec",)], kmm=[(2, NT, 0, 384)], route=(0, 256)),
        dict(wait=[wq], perm=wq[1:], kmm=[(2, NT, 384, 512)], route=(256, 512), mm=mm((Q, 0))),
        dict(wait=[wv, x1], perm=wv[1:], route=(512, 896), mm=mm((Q, 256), (V, 0), (V, 256)), halo=True),
        stage(512, 256, wait=[x2, ("wo",)], route=(896, 1536)),
        stage(768, 512, route=(1536, S), select=True, fused=True),
        stage(1024, 752, wait=[("gu",)], gate_up=(0, 36)),
        stage(1280, 976, gate_up=(36, 72), perm_wo=True, fused=True),
        stage(1536, 1232, wait=[("down",)], gate_up=(72, F // 16)),
        stage(1792, 1504, gates=(0, 768), down=True, fused=True),
        dict(patch=True, gates=(768, 1536), out=[(0, 256), (256, 256), (512, 256)], att=1776),
        dict(gates=(1536, 1920), out=[(768, 256), (1024, 256), (1280, 256)], att=S),
        dict(gates=(1920, S), out=[(1536, 256), (1792, 128)]),
        dict(out=[(1920, 128)]),
    ]


_DMA, _REGIONS = _plan()
_OUTS = [o for r in _REGIONS for o in r.get("out", ())]
_IN_SEMS = len(_DMA) + NT + 1


def _tree(f, xs):
    while len(xs) > 1:
        xs = [f(xs[k], xs[k + 1]) if k + 1 < len(xs) else xs[k] for k in range(0, len(xs), 2)]
    return xs[0]


def _rows(r0, n):
    return pl.ds(r0 // 2, n // 2)


def _bf16(words):
    return pltpu.bitcast(words, BF16)


def _words(x):
    return pltpu.bitcast(x.astype(BF16), I32)


def _ordered(bits):
    return jnp.where(bits < 0, bits ^ np.int32(0x7FFF0000), bits)


def _kernel(x_hbm, wqkv_hbm, wo_hbm, wr_hbm, wg_hbm, wu_hbm, wd_hbm, gw_hbm, out_hbm,
            x, wraw, wp, wo_raw, wop, wg, wu, wd, wr, gw,
            qkv, att_out, out, gate, gate_rep, xsel, hidden, in_sem, out_sem, barrier):
    x_h, wqkv_h, out_h = (r.bitcast(I32) for r in (x_hbm, wqkv_hbm, out_hbm))

    copies, n_sem = {}, 0
    for d in _DMA:
        if d[0] == "w":
            rows = _rows(d[2] * 128, (d[3] - d[2]) * 128)
            pairs = [(wqkv_h.at[rows, pl.ds(d[1] * D, D)], wraw.at[d[1], rows])]
        elif d[0] == "xc":
            blk = (_rows(0, 512), pl.ds(d[1] * 128, (d[2] - d[1]) * 128))
            pairs = [(x_h.at[blk], x.at[blk])]
        elif d[0] == "x":
            rows = _rows(d[1], d[2] - d[1])
            pairs = [(x_h.at[rows], x.at[rows])]
        elif d[0] == "vec":
            pairs = [(wr_hbm, wr), (gw_hbm, gw)]
        elif d[0] == "wo":
            pairs = [(wo_hbm.bitcast(I32).at[:, pl.ds(j * 128, 128)], wo_raw.at[j]) for j in range(NT)]
        elif d[0] == "gu":
            pairs = [(wg_hbm.bitcast(I32), wg), (wu_hbm.bitcast(I32), wu)]
        else:
            pairs = [(wd_hbm.bitcast(I32), wd)]
        copies[d] = [pltpu.make_async_copy(a, b, in_sem.at[n_sem + k]) for k, (a, b) in enumerate(pairs)]
        n_sem += len(pairs)
        for c in copies[d]:
            c.start()
    out_copies = {o: pltpu.make_async_copy(out.at[_rows(*o)], out_h.at[_rows(*o)], out_sem.at[k])
                  for k, o in enumerate(_OUTS)}

    lane = lax.broadcasted_iota(I32, (8, 128), 1)
    sub = lax.broadcasted_iota(I32, (8, 128), 0)

    def permute_wqkv(s, k0, k1):
        for jp in range(NT):
            src = (DH * (lane & 31) + 4 * jp + (lane >> 5)) & 127
            tile = (DH * ((13 * ((lane >> 2) - jp)) & 31) + 4 * jp + (lane & 3)) >> 7
            for r in range(k0 * 8, k1 * 8):
                rows = pl.ds(r * 8, 8)
                acc = wraw[s, rows, pl.ds(0, 128)]
                for j in range(1, NT):
                    acc = jnp.where(tile == j, wraw[s, rows, pl.ds(j * 128, 128)], acc)
                wp[rows, pl.ds(s * D + jp * 128, 128)] = jnp.take_along_axis(acc, src, axis=1)

    def permute_wo():
        for j in range(NT):
            cols = pl.ds(j * 128, 128)
            for i in range(DH // 2):
                even = wo_raw[j, pl.ds(i, H // 2, stride=DH), :]
                odd = wo_raw[j, pl.ds(DH // 2 + i, H // 2, stride=DH), :]
                wop[pl.ds(i * 32, 16), cols] = (even & 0xFFFF) | (odd << 16)
                wop[pl.ds(i * 32 + 16, 16), cols] = lax.shift_right_logical(even, 16) | (odd & HI)

    def project(s, r0, k0=0, k1=NT):
        y = jnp.dot(_bf16(x[_rows(r0, MM), k0 * 128:k1 * 128]), _bf16(wp[k0 * 64:k1 * 64, s * D:(s + 1) * D]),
                    preferred_element_type=F32)
        if s == Q:
            y = y * Q_SCALE
        for j in range(NT):
            dst = (s * NT + j, pl.ds(HALO + r0, MM), slice(None))
            yj = y[:, j * 128:(j + 1) * 128]
            qkv[dst] = qkv[dst] + yj if k0 else yj

    att_done = 0

    def attention():
        nonlocal att_done
        lags, n = (6, 12, 18), S // 8 * W
        half, quarter, logit, weight, acc = {}, {}, {}, {}, [None] * NT
        for t in range(n + lags[2] + W):
            yield min(S, (t // W + 1) * 8)
            if t < n:
                g, w = divmod(t, W)
                if w == 0:
                    q = [qkv[Q * NT + j, pl.ds(HALO + g * 8, 8), :] for j in range(NT)]
                rows = pl.ds(HALO + g * 8 - DIL * w, 8)
                a = q[0] * qkv[K * NT, rows, :]
                for j in range(1, NT):
                    a = a + q[j] * qkv[K * NT + j, rows, :]
                half[t] = (a, pltpu.roll(a, 64, 1))
            u = t - lags[0]
            if 0 <= u < n:
                a, b = half.pop(u)
                a = a + b
                quarter[u] = (a, pltpu.roll(a, 32, 1))
            u = t - lags[1]
            if 0 <= u < n:
                g, w = divmod(u, W)
                a, b = quarter.pop(u)
                a = a + b
                if g * 8 < DIL * w:
                    a = jnp.where(sub + g * 8 >= DIL * w, a, MASKED)
                logit[u] = a
                if w == W - 1:
                    row = [logit.pop(g * W + k) for k in range(W)]
                    top = _tree(jnp.maximum, row)
                    for k in range(W):
                        weight[g * W + k] = jnp.exp2(row[k] - top)
            u = t - lags[2] - (W - 1)
            if 0 <= u < n:
                g, w = divmod(u, W)
                if w == 0:
                    den = _tree(jnp.add, [weight[g * W + k] for k in range(W)])
                    inv = pl.reciprocal(den, approx=True)
                if w == W // 2:
                    inv = inv * (2.0 - den * inv)
                e = weight.pop(u)
                rows = pl.ds(HALO + g * 8 - DIL * w, 8)
                for j in range(NT):
                    p = e * qkv[V * NT + j, rows, :]
                    acc[j] = p if w == 0 else acc[j] + p
                if w == W - 1:
                    o = [a * inv for a in acc]
                    if g % 2 == 0:
                        held = o
                    else:
                        for j in range(NT):
                            att_out[_rows((g - 1) * 8, 16), pl.ds(j * 128, 128)] = _words(
                                jnp.concatenate([held[j], o[j]], axis=0))
                        att_done = (g + 1) * 8

    score = [jnp.zeros((8, 128), F32)] * 2
    gate_logit = list(score)
    vecs, picked = [], {}

    def route(r0, r1):
        if not vecs:
            vecs.extend(jnp.broadcast_to(v[...].astype(F32).reshape(1, D), (8, D)) for v in (wr, gw))
        for g in range(r0 // 16, r1 // 16):
            xf = _bf16(x[_rows(g * 16, 16), :]).astype(F32)
            for p in range(2):
                c, l = divmod(2 * g + p, 128)
                for dst, vec in zip((score, gate_logit), vecs):
                    val = jnp.sum(xf[8 * p:8 * p + 8] * vec, axis=1, keepdims=True)
                    dst[c] = jnp.where(lane == l, val, dst[c])

    def token_group(t):
        return pl.ds(pl.multiple_of((t >> 4) << 3, 8), 8), lax.broadcasted_iota(I32, (16, D), 0) == (t & 15)

    def select():
        keys = []
        for c in range(2):
            gate[c] = jax.nn.sigmoid(gate_logit[c])
        for c in range(2):
            r = score[c].astype(BF16).astype(F32)
            r = jnp.where(r == 0, np.float32(0), r)
            key = jnp.where(r != r, INT_MIN, _ordered(pltpu.bitcast(r, I32)))
            keys.append(key | (S - 1 - (1024 * c + 8 * lane + sub)))
        k1 = jnp.max(jnp.maximum(*keys))
        k2 = jnp.max(jnp.maximum(*[jnp.where(k == k1, INT_MIN, k) for k in keys]))
        picked["keys"] = (k1, k2)
        picked["rows"] = [S - 1 - (k & (S - 1)) for k in (k1, k2)]
        for c, t in enumerate(picked["rows"]):
            rows, here = token_group(t)
            row = jnp.sum(jnp.where(here, _bf16(x[rows, :]).astype(F32), 0.0), axis=0, keepdims=True)
            xsel[c] = jnp.broadcast_to(row, (8, D))

    pre = {}

    def gate_up(l):
        for m, w_ref in enumerate((wg, wu)):
            ww = w_ref[pl.ds(l * 8, 8), :]
            for p, wf in enumerate((ww << 16, ww & HI)):
                here = lane - 2 * sub == 16 * (l % 8) + p
                for c in range(2):
                    val = jnp.sum(pltpu.bitcast(wf, F32) * xsel[c], axis=1, keepdims=True)
                    pre[m, c] = jnp.where(here, val, pre.get((m, c), np.float32(0)))
        if l % 8 == 7 or l == F // 16 - 1:
            h = [jax.nn.silu(pre.pop((0, c))) * pre.pop((1, c)) for c in range(2)]
            hidden[:, pl.ds(l // 8 * 128, 128)] = _words(jnp.concatenate(h, axis=0))

    def down():
        y = jnp.dot(_bf16(hidden[:, pl.ds(0, F)]), _bf16(wd[...]), preferred_element_type=F32)
        picked["update"] = []
        for c, k in enumerate(picked["keys"]):
            r = jax.nn.sigmoid(pltpu.bitcast(_ordered(jnp.full((1, 128), k & HI, I32)), F32))
            yc = jnp.sum(y[8 * c:8 * c + 8], axis=0, keepdims=True)
            picked["update"].append(yc * jnp.concatenate([r] * NT, axis=1))

    def patch():
        for t, upd in zip(picked["rows"], picked["update"]):
            rows, here = token_group(t)
            blk = _bf16(x[rows, :]).astype(F32)
            x[rows, :] = _words(jnp.where(here, blk + upd, blk))

    def mix(r0, n):
        rows = _rows(r0, n)
        a = jnp.dot(_bf16(att_out[rows, :]), _bf16(wop[...]), preferred_element_type=F32)
        b = _bf16(x[rows, :]).astype(F32)
        g = jnp.concatenate([gate_rep[pl.ds(r0, n), :]] * NT, axis=1)
        out[rows, :] = _words(b + g * (a - b))

    for j in range(NT):
        qkv[K * NT + j, pl.ds(0, HALO), :] = jnp.zeros((HALO, 128), F32)
    steps = attention()
    need = next(steps)
    for r in _REGIONS:
        for d in r.get("wait", ()):
            for c in copies[d]:
                c.wait()
        if not r.get("fused") and not r.get("wait"):
            pl.semaphore_signal(barrier, 1)
            pl.semaphore_wait(barrier, 1)
        if r.get("patch"):
            patch()
        if "perm" in r:
            permute_wqkv(*r["perm"])
        for k0, k1, r0, r1 in r.get("kmm", ()):
            for a in range(r0, r1, MM):
                project(K, a, k0, k1)
        if "route" in r:
            route(*r["route"])
        for l in range(*r.get("gate_up", (0,))):
            gate_up(l)
        if "gates" in r:
            compact = [gate[0], gate[1]]
            for m in range(r["gates"][0] // 8, r["gates"][1] // 8):
                c, l = divmod(m, 128)
                gate_rep[pl.ds(m * 8, 8), :] = jnp.broadcast_to(compact[c][:, l:l + 1], (8, 128))
        if r.get("perm_wo"):
            permute_wo()
        for s, r0 in r.get("mm", ()):
            project(s, r0)
        if r.get("halo"):
            for j in range(NT):
                first = qkv[V * NT + j, pl.ds(HALO, 1), :]
                qkv[V * NT + j, pl.ds(0, HALO), :] = jnp.broadcast_to(first, (HALO, 128))
        for r0, n in r.get("out", ()):
            assert att_done >= r0 + n
            mix(r0, n)
        while need is not None and need <= r.get("att", 0):
            need = next(steps, None)
        if r.get("select"):
            select()
        if r.get("down"):
            down()
        for o in r.get("out", ()):
            out_copies[o].start()
    for o in _OUTS:
        out_copies[o].wait()


@jax.jit
def pallas_gated_mix__sliding_local_dilated__moe_arch_mod__prompt_kernel(
    A_x: jax.Array,
    A_wqkv: jax.Array,
    A_wo: jax.Array,
    B_x: jax.Array,
    B_w_r: jax.Array,
    B_w_gate: jax.Array,
    B_w_up: jax.Array,
    B_w_down: jax.Array,
    gate_w: jax.Array,
):
    del B_x
    hbm = pl.BlockSpec(memory_space=pltpu.HBM)
    out = pl.pallas_call(
        _kernel,
        out_shape=jax.ShapeDtypeStruct((S, D), BF16),
        in_specs=[hbm] * 8,
        out_specs=hbm,
        scratch_shapes=[
            pltpu.VMEM((S // 2, D), I32),
            pltpu.VMEM((3, D // 2, D), I32),
            pltpu.VMEM((D // 2, 3 * D), I32),
            pltpu.VMEM((NT, D // 2, 128), I32),
            pltpu.VMEM((D // 2, D), I32),
            pltpu.VMEM((F // 2, D), I32),
            pltpu.VMEM((F // 2, D), I32),
            pltpu.VMEM((F // 2, D), I32),
            pltpu.VMEM((D,), BF16),
            pltpu.VMEM((D,), BF16),
            pltpu.VMEM((3 * NT, HALO + S, 128), F32),
            pltpu.VMEM((S // 2, D), I32),
            pltpu.VMEM((S // 2, D), I32),
            pltpu.VMEM((2, 8, 128), F32),
            pltpu.VMEM((S, 128), F32),
            pltpu.VMEM((2, 8, D), F32),
            pltpu.VMEM((8, pl.cdiv(F, 128) * 128), I32),
            pltpu.SemaphoreType.DMA((_IN_SEMS,)),
            pltpu.SemaphoreType.DMA((len(_OUTS),)),
            pltpu.SemaphoreType.REGULAR,
        ],
        compiler_params=pltpu.CompilerParams(vmem_limit_bytes=64 * 2**20),
    )(A_x.reshape(S, D), A_wqkv, A_wo, B_w_r, B_w_gate.T, B_w_up.T, B_w_down, gate_w)
    return out.reshape(1, S, D)
```

```python
import jax
import jax.numpy as jnp
import numpy as np
from jax import lax
from jax.experimental import pallas as pl
from jax.experimental.pallas import tpu as pltpu

S, D, H, DH, W, DIL, F = 2048, 640, 32, 20, 8, 2, 1728
NT = D // 128
HALO = 16
MM = 128
Q, K, V = 0, 1, 2
F32, BF16, I32 = jnp.float32, jnp.bfloat16, jnp.int32
HI = np.int32(-65536)
INT_MIN = np.int32(-2**31)
Q_SCALE = np.float32(DH ** -0.5 * np.log2(np.e))
MASKED = np.float32(-1e9 * np.log2(np.e))


def _plan():
    xa, wa, xb, wb = ("xc", 0, 2), ("w", K, 0, 2), ("xc", 2, NT), ("w", K, 2, NT)
    wq, wv, x1, x2 = ("w", Q, 0, NT), ("w", V, 0, NT), ("x", 512, 832), ("x", 832, S)
    dma = [wa, xa, wb, xb, ("vec",), wq, wv, x1, x2, ("gu",), ("down",), ("wo",)]

    def mm(*blocks):
        return [(s, r0 + a) for s, r0 in blocks for a in range(0, 256, MM)]

    def stage(r0, att, **kw):
        return dict(mm=mm((V, r0), (Q, r0), (K, r0)), att=att, **kw)

    return dma, [
        dict(wait=[wa], perm=wa[1:]),
        dict(wait=[xa], kmm=[(0, 2, 0, 512)]),
        dict(wait=[wb], perm=wb[1:]),
        dict(wait=[xb, ("vec",)], kmm=[(2, NT, 0, 384)], route=(0, 256)),
        dict(wait=[wq], perm=wq[1:], kmm=[(2, NT, 384, 512)], route=(256, 512), mm=mm((Q, 0))),
        dict(wait=[wv, x1], perm=wv[1:], route=(512, 832), mm=mm((Q, 256), (V, 0), (V, 256)), halo=True),
        stage(512, 256, wait=[x2], route=(832, 1536)),
        stage(768, 512, route=(1536, S), select=True, fused=True),
        stage(1024, 752, wait=[("gu",)], gate_up=(0, 34)),
        stage(1280, 976, gate_up=(34, 70), fused=True),
        stage(1536, 1232, wait=[("down",), ("wo",)], gate_up=(70, F // 16)),
        stage(1792, 1504, gates=(0, 768), down=True, perm_wo=True, fused=True),
        dict(patch=True, gates=(768, 1536), out=[(0, 256), (256, 256), (512, 256)], att=1776),
        dict(gates=(1536, 1920), out=[(768, 256), (1024, 256), (1280, 256)], att=S),
        dict(gates=(1920, S), out=[(1536, 256), (1792, 128)]),
        dict(out=[(1920, 128)]),
    ]


_DMA, _REGIONS = _plan()
_OUTS = [o for r in _REGIONS for o in r.get("out", ())]
_IN_SEMS = len(_DMA) + NT + 1


def _tree(f, xs):
    while len(xs) > 1:
        xs = [f(xs[k], xs[k + 1]) if k + 1 < len(xs) else xs[k] for k in range(0, len(xs), 2)]
    return xs[0]


def _rows(r0, n):
    return pl.ds(r0 // 2, n // 2)


def _bf16(words):
    return pltpu.bitcast(words, BF16)


def _words(x):
    return pltpu.bitcast(x.astype(BF16), I32)


def _ordered(bits):
    return jnp.where(bits < 0, bits ^ np.int32(0x7FFF0000), bits)


def _kernel(x_hbm, wqkv_hbm, wo_hbm, wr_hbm, wg_hbm, wu_hbm, wd_hbm, gw_hbm, out_hbm,
            x, wraw, wp, wo_raw, wop, wg, wu, wd, wr, gw,
            qkv, att_out, out, gate, gate_rep, xsel, hidden, in_sem, out_sem, barrier):
    x_h, wqkv_h, out_h = (r.bitcast(I32) for r in (x_hbm, wqkv_hbm, out_hbm))

    copies, n_sem = {}, 0
    for d in _DMA:
        if d[0] == "w":
            rows = _rows(d[2] * 128, (d[3] - d[2]) * 128)
            pairs = [(wqkv_h.at[rows, pl.ds(d[1] * D, D)], wraw.at[d[1], rows])]
        elif d[0] == "xc":
            blk = (_rows(0, 512), pl.ds(d[1] * 128, (d[2] - d[1]) * 128))
            pairs = [(x_h.at[blk], x.at[blk])]
        elif d[0] == "x":
            rows = _rows(d[1], d[2] - d[1])
            pairs = [(x_h.at[rows], x.at[rows])]
        elif d[0] == "vec":
            pairs = [(wr_hbm, wr), (gw_hbm, gw)]
        elif d[0] == "wo":
            pairs = [(wo_hbm.bitcast(I32).at[:, pl.ds(j * 128, 128)], wo_raw.at[j]) for j in range(NT)]
        elif d[0] == "gu":
            pairs = [(wg_hbm.bitcast(I32), wg), (wu_hbm.bitcast(I32), wu)]
        else:
            pairs = [(wd_hbm.bitcast(I32), wd)]
        copies[d] = [pltpu.make_async_copy(a, b, in_sem.at[n_sem + k]) for k, (a, b) in enumerate(pairs)]
        n_sem += len(pairs)
        for c in copies[d]:
            c.start()
    out_copies = {o: pltpu.make_async_copy(out.at[_rows(*o)], out_h.at[_rows(*o)], out_sem.at[k])
                  for k, o in enumerate(_OUTS)}

    lane = lax.broadcasted_iota(I32, (8, 128), 1)
    sub = lax.broadcasted_iota(I32, (8, 128), 0)

    def permute_wqkv(s, k0, k1):
        for jp in range(NT):
            src = (DH * (lane & 31) + 4 * jp + (lane >> 5)) & 127
            tile = (DH * ((13 * ((lane >> 2) - jp)) & 31) + 4 * jp + (lane & 3)) >> 7
            for r in range(k0 * 8, k1 * 8):
                rows = pl.ds(r * 8, 8)
                acc = wraw[s, rows, pl.ds(0, 128)]
                for j in range(1, NT):
                    acc = jnp.where(tile == j, wraw[s, rows, pl.ds(j * 128, 128)], acc)
                wp[rows, pl.ds(s * D + jp * 128, 128)] = jnp.take_along_axis(acc, src, axis=1)

    def permute_wo():
        for j in range(NT):
            cols = pl.ds(j * 128, 128)
            for i in range(DH // 2):
                even = wo_raw[j, pl.ds(i, H // 2, stride=DH), :]
                odd = wo_raw[j, pl.ds(DH // 2 + i, H // 2, stride=DH), :]
                wop[pl.ds(i * 32, 16), cols] = (even & 0xFFFF) | (odd << 16)
                wop[pl.ds(i * 32 + 16, 16), cols] = lax.shift_right_logical(even, 16) | (odd & HI)

    def project(s, r0, k0=0, k1=NT):
        y = jnp.dot(_bf16(x[_rows(r0, MM), k0 * 128:k1 * 128]), _bf16(wp[k0 * 64:k1 * 64, s * D:(s + 1) * D]),
                    preferred_element_type=F32)
        if s == Q:
            y = y * Q_SCALE
        for j in range(NT):
            dst = (s * NT + j, pl.ds(HALO + r0, MM), slice(None))
            yj = y[:, j * 128:(j + 1) * 128]
            qkv[dst] = qkv[dst] + yj if k0 else yj

    att_done = 0

    def attention():
        nonlocal att_done
        lags, n = (6, 12, 18), S // 8 * W
        half, quarter, logit, weight, acc = {}, {}, {}, {}, [None] * NT
        for t in range(n + lags[2] + W):
            yield min(S, (t // W + 1) * 8)
            if t < n:
                g, w = divmod(t, W)
                if w == 0:
                    q = [qkv[Q * NT + j, pl.ds(HALO + g * 8, 8), :] for j in range(NT)]
                rows = pl.ds(HALO + g * 8 - DIL * w, 8)
                a = q[0] * qkv[K * NT, rows, :]
                for j in range(1, NT):
                    a = a + q[j] * qkv[K * NT + j, rows, :]
                half[t] = (a, pltpu.roll(a, 64, 1))
            u = t - lags[0]
            if 0 <= u < n:
                a, b = half.pop(u)
                a = a + b
                quarter[u] = (a, pltpu.roll(a, 32, 1))
            u = t - lags[1]
            if 0 <= u < n:
                g, w = divmod(u, W)
                a, b = quarter.pop(u)
                a = a + b
                if g * 8 < DIL * w:
                    a = jnp.where(sub + g * 8 >= DIL * w, a, MASKED)
                logit[u] = a
                if w == W - 1:
                    row = [logit.pop(g * W + k) for k in range(W)]
                    top = _tree(jnp.maximum, row)
                    for k in range(W):
                        weight[g * W + k] = jnp.exp2(row[k] - top)
            u = t - lags[2] - (W - 1)
            if 0 <= u < n:
                g, w = divmod(u, W)
                if w == 0:
                    den = _tree(jnp.add, [weight[g * W + k] for k in range(W)])
                    inv = pl.reciprocal(den, approx=True)
                if w == W // 2:
                    inv = inv * (2.0 - den * inv)
                e = weight.pop(u)
                rows = pl.ds(HALO + g * 8 - DIL * w, 8)
                for j in range(NT):
                    p = e * qkv[V * NT + j, rows, :]
                    acc[j] = p if w == 0 else acc[j] + p
                if w == W - 1:
                    o = [a * inv for a in acc]
                    if g % 2 == 0:
                        held = o
                    else:
                        for j in range(NT):
                            att_out[_rows((g - 1) * 8, 16), pl.ds(j * 128, 128)] = _words(
                                jnp.concatenate([held[j], o[j]], axis=0))
                        att_done = (g + 1) * 8

    score = [jnp.zeros((8, 128), F32)] * 2
    gate_logit = list(score)
    vecs, picked = [], {}

    def route(r0, r1):
        if not vecs:
            vecs.extend(jnp.broadcast_to(v[...].astype(F32).reshape(1, D), (8, D)) for v in (wr, gw))
        for g in range(r0 // 16, r1 // 16):
            xf = _bf16(x[_rows(g * 16, 16), :]).astype(F32)
            for p in range(2):
                c, l = divmod(2 * g + p, 128)
                for dst, vec in zip((score, gate_logit), vecs):
                    val = jnp.sum(xf[8 * p:8 * p + 8] * vec, axis=1, keepdims=True)
                    dst[c] = jnp.where(lane == l, val, dst[c])

    def token_group(t):
        return pl.ds(pl.multiple_of((t >> 4) << 3, 8), 8), lax.broadcasted_iota(I32, (16, D), 0) == (t & 15)

    def select():
        keys = []
        for c in range(2):
            gate[c] = jax.nn.sigmoid(gate_logit[c])
        for c in range(2):
            r = score[c].astype(BF16).astype(F32)
            r = jnp.where(r == 0, np.float32(0), r)
            key = jnp.where(r != r, INT_MIN, _ordered(pltpu.bitcast(r, I32)))
            keys.append(key | (S - 1 - (1024 * c + 8 * lane + sub)))
        k1 = jnp.max(jnp.maximum(*keys))
        k2 = jnp.max(jnp.maximum(*[jnp.where(k == k1, INT_MIN, k) for k in keys]))
        picked["keys"] = (k1, k2)
        picked["rows"] = [S - 1 - (k & (S - 1)) for k in (k1, k2)]
        for c, t in enumerate(picked["rows"]):
            rows, here = token_group(t)
            row = jnp.sum(jnp.where(here, _bf16(x[rows, :]).astype(F32), 0.0), axis=0, keepdims=True)
            xsel[c] = jnp.broadcast_to(row, (8, D))

    pre = {}

    def gate_up(l):
        for m, w_ref in enumerate((wg, wu)):
            ww = w_ref[pl.ds(l * 8, 8), :]
            for p, wf in enumerate((ww << 16, ww & HI)):
                here = lane - 2 * sub == 16 * (l % 8) + p
                for c in range(2):
                    val = jnp.sum(pltpu.bitcast(wf, F32) * xsel[c], axis=1, keepdims=True)
                    pre[m, c] = jnp.where(here, val, pre.get((m, c), np.float32(0)))
        if l % 8 == 7 or l == F // 16 - 1:
            h = [jax.nn.silu(pre.pop((0, c))) * pre.pop((1, c)) for c in range(2)]
            hidden[:, pl.ds(l // 8 * 128, 128)] = _words(jnp.concatenate(h, axis=0))

    def down():
        y = jnp.dot(_bf16(hidden[:, pl.ds(0, F)]), _bf16(wd[...]), preferred_element_type=F32)
        picked["update"] = []
        for c, k in enumerate(picked["keys"]):
            r = jax.nn.sigmoid(pltpu.bitcast(_ordered(jnp.full((1, 128), k & HI, I32)), F32))
            yc = jnp.sum(y[8 * c:8 * c + 8], axis=0, keepdims=True)
            picked["update"].append(yc * jnp.concatenate([r] * NT, axis=1))

    def patch():
        for t, upd in zip(picked["rows"], picked["update"]):
            rows, here = token_group(t)
            blk = _bf16(x[rows, :]).astype(F32)
            x[rows, :] = _words(jnp.where(here, blk + upd, blk))

    def mix(r0, n):
        rows = _rows(r0, n)
        a = jnp.dot(_bf16(att_out[rows, :]), _bf16(wop[...]), preferred_element_type=F32)
        b = _bf16(x[rows, :]).astype(F32)
        g = jnp.concatenate([gate_rep[pl.ds(r0, n), :]] * NT, axis=1)
        out[rows, :] = _words(b + g * (a - b))

    for j in range(NT):
        qkv[K * NT + j, pl.ds(0, HALO), :] = jnp.zeros((HALO, 128), F32)
    steps = attention()
    need = next(steps)
    for r in _REGIONS:
        for d in r.get("wait", ()):
            for c in copies[d]:
                c.wait()
        if not r.get("fused") and not r.get("wait"):
            pl.semaphore_signal(barrier, 1)
            pl.semaphore_wait(barrier, 1)
        if r.get("patch"):
            patch()
        if "perm" in r:
            permute_wqkv(*r["perm"])
        for k0, k1, r0, r1 in r.get("kmm", ()):
            for a in range(r0, r1, MM):
                project(K, a, k0, k1)
        if "route" in r:
            route(*r["route"])
        for l in range(*r.get("gate_up", (0,))):
            gate_up(l)
        if "gates" in r:
            compact = [gate[0], gate[1]]
            for m in range(r["gates"][0] // 8, r["gates"][1] // 8):
                c, l = divmod(m, 128)
                gate_rep[pl.ds(m * 8, 8), :] = jnp.broadcast_to(compact[c][:, l:l + 1], (8, 128))
        if r.get("perm_wo"):
            permute_wo()
        for s, r0 in r.get("mm", ()):
            project(s, r0)
        if r.get("halo"):
            for j in range(NT):
                first = qkv[V * NT + j, pl.ds(HALO, 1), :]
                qkv[V * NT + j, pl.ds(0, HALO), :] = jnp.broadcast_to(first, (HALO, 128))
        for r0, n in r.get("out", ()):
            assert att_done >= r0 + n
            mix(r0, n)
        while need is not None and need <= r.get("att", 0):
            need = next(steps, None)
        if r.get("select"):
            select()
        if r.get("down"):
            down()
        for o in r.get("out", ()):
            out_copies[o].start()
    for o in _OUTS:
        out_copies[o].wait()


@jax.jit
def pallas_gated_mix__sliding_local_dilated__moe_arch_mod__prompt_kernel(
    A_x: jax.Array,
    A_wqkv: jax.Array,
    A_wo: jax.Array,
    B_x: jax.Array,
    B_w_r: jax.Array,
    B_w_gate: jax.Array,
    B_w_up: jax.Array,
    B_w_down: jax.Array,
    gate_w: jax.Array,
):
    del B_x
    hbm = pl.BlockSpec(memory_space=pltpu.HBM)
    out = pl.pallas_call(
        _kernel,
        out_shape=jax.ShapeDtypeStruct((S, D), BF16),
        in_specs=[hbm] * 8,
        out_specs=hbm,
        scratch_shapes=[
            pltpu.VMEM((S // 2, D), I32),
            pltpu.VMEM((3, D // 2, D), I32),
            pltpu.VMEM((D // 2, 3 * D), I32),
            pltpu.VMEM((NT, D // 2, 128), I32),
            pltpu.VMEM((D // 2, D), I32),
            pltpu.VMEM((F // 2, D), I32),
            pltpu.VMEM((F // 2, D), I32),
            pltpu.VMEM((F // 2, D), I32),
            pltpu.VMEM((D,), BF16),
            pltpu.VMEM((D,), BF16),
            pltpu.VMEM((3 * NT, HALO + S, 128), F32),
            pltpu.VMEM((S // 2, D), I32),
            pltpu.VMEM((S // 2, D), I32),
            pltpu.VMEM((2, 8, 128), F32),
            pltpu.VMEM((S, 128), F32),
            pltpu.VMEM((2, 8, D), F32),
            pltpu.VMEM((8, pl.cdiv(F, 128) * 128), I32),
            pltpu.SemaphoreType.DMA((_IN_SEMS,)),
            pltpu.SemaphoreType.DMA((len(_OUTS),)),
            pltpu.SemaphoreType.REGULAR,
        ],
        compiler_params=pltpu.CompilerParams(vmem_limit_bytes=64 * 2**20),
    )(A_x.reshape(S, D), A_wqkv, A_wo, B_w_r, B_w_gate.T, B_w_up.T, B_w_down, gate_w)
    return out.reshape(1, S, D)
```
